```python
import jax
import jax.numpy as jnp

def _softmax(x, axis=-1):
    return jax.nn.softmax(x, axis=axis)
def _gelu(x):
    return jax.nn.gelu(x, approximate=True)
def _silu(x):
    return jax.nn.silu(x)
def _sigmoid(x):
    return jax.nn.sigmoid(x)
def _layernorm(x, axis=-1, eps=1e-5):
    m = jnp.mean(x, axis=axis, keepdims=True)
    v = jnp.var(x, axis=axis, keepdims=True)
    return (x - m) / jnp.sqrt(v + eps)
def _scatter_add(tgt, idx, src, axis=0):
    return tgt.at[idx].add(src)
def _segment_sum(src, seg, n):
    return jax.ops.segment_sum(src, seg, n)
class _Rng:
    def __init__(self, key):
        self._k = key
    def _next(self):
        self._k, sub = jax.random.split(self._k)
        return sub
    def normal(self, shape):
        return jax.random.normal(self._next(), shape, dtype=jnp.bfloat16)
    def randint(self, lo, hi, shape):
        return jax.random.randint(self._next(), shape, lo, hi, dtype=jnp.int32)
    def uniform(self, shape, lo=0.0, hi=1.0):
        return jax.random.uniform(self._next(), shape, jnp.bfloat16, lo, hi)
    def permutation(self, n):
        return jax.random.permutation(self._next(), n)


kernel_name = 'parallel_sum__sliding_local_dilated__mixer_token_mlp__prompt'

def setup_inputs():
    _rng = _Rng(jax.random.key(int.from_bytes(__import__("os").urandom(4), "little")))
    _w = (lambda a: (lambda t: t.astype(jnp.bfloat16) if jnp.issubdtype(t.dtype, jnp.floating) else t)(jnp.asarray(a)))
    def _A_setup():
        B, S, D = 1, 2048, 448
        return {
            "x": _w((lambda *s: _rng.normal(s) * 0.05)(B, S, D)),
            "wqkv": _w((lambda *s: _rng.normal(s) * 0.05)(D, 3 * D)),
            "wo": _w((lambda *s: _rng.normal(s) * 0.05)(D, D)),
        }
    _A_in = _A_setup()

    def _B_setup():
        B, S, D, F = 1, 2048, 448, 1792
        return {
            "x": _w((lambda *s: _rng.normal(s) * 0.05)(B, S, D)),
            "w1": _w((lambda *s: _rng.normal(s) * 0.05)(S, F) * (S ** -0.5)),
            "b1": _w((lambda *s: _rng.normal(s) * 0.05)(F) * 0.02),
            "w2": _w((lambda *s: _rng.normal(s) * 0.05)(F, S) * (F ** -0.5)),
            "b2": _w((lambda *s: _rng.normal(s) * 0.05)(S) * 0.02),
        }
    _B_in = _B_setup()

    return {
        "A_x": _A_in["x"],
        "A_wqkv": _A_in["wqkv"],
        "A_wo": _A_in["wo"],
        "B_x": _B_in["x"],
        "B_w1": _B_in["w1"],
        "B_b1": _B_in["b1"],
        "B_w2": _B_in["w2"],
        "B_b2": _B_in["b2"],
    }

def reference(A_x, A_wqkv, A_wo, B_x, B_w1, B_b1, B_w2, B_b2):
    def _A_ref(x, wqkv, wo):
        B, S, D = x.shape
        H = 16; Dh = D // H
        W, dil = 8, 2
        qkv = (lambda x, *d: x.transpose(*d))((x @ wqkv).reshape(B, S, 3, H, Dh), 2, 0, 3, 1, 4)
        q, k, v = qkv[0], qkv[1], qkv[2]
        scale = Dh ** -0.5
        pos = jnp.arange(S)
        off = jnp.arange(W) * dil
        idx = pos[:, None] - off[None, :]
        mask = idx >= 0
        idx_c = jnp.where(mask, idx, 0).reshape(-1)
        kg = k[:, :, idx_c, :].reshape(B, H, S, W, Dh)
        vg = v[:, :, idx_c, :].reshape(B, H, S, W, Dh)
        logits = jnp.einsum("bhsd,bhswd->bhsw", q, kg) * scale
        logits = jnp.where(mask[None, None, :, :], logits, -1e9)
        attn = _softmax(logits, axis=-1)
        o = jnp.einsum("bhsw,bhswd->bhsd", attn, vg)
        return (lambda x, *d: x.transpose(*d))(o, 0, 2, 1, 3).reshape(B, S, D) @ wo

    def _B_ref(x, w1, b1, w2, b2):
        B, S, D = x.shape
        h = _layernorm(x, axis=-1)
        u = jnp.einsum("bsd,sf->bdf", h, w1) + b1
        u = _gelu(u)
        y = jnp.einsum("bdf,fs->bds", u, w2) + b2
        return (lambda x, *d: x.transpose(*d))(y, 0, 2, 1)

    x = A_x
    xn = _layernorm(x, axis=-1)
    return x + _A_ref(xn, A_wqkv, A_wo) + _B_ref(xn, B_w1, B_b1, B_w2, B_b2)
```

```python
import functools
import jax
import jax.numpy as jnp
import jax.experimental.pallas as pl
import jax.experimental.pallas.tpu as pltpu

S, D, H, DH, F = 2048, 448, 16, 28, 1792
W, DIL = 8, 2
C = 256
NC = S // C
EPS = 1e-5
SCALE = DH ** -0.5
BF, F32 = jnp.bfloat16, jnp.float32


def _gelu(x):
    c0 = 0.7978845608028654
    inner = c0 * (x + 0.044715 * (x * x * x))
    return 0.5 * x * (1.0 + jnp.tanh(inner))


def _ln_cols(x):
    m = jnp.sum(x, axis=0, keepdims=True) * (1.0 / D)
    xc = x - m
    v = jnp.sum(xc * xc, axis=0, keepdims=True) * (1.0 / D)
    return xc * jax.lax.rsqrt(v + EPS)


def _rot256(y, shift):
    return jnp.concatenate(
        [pltpu.roll(y[:, :128], shift, axis=1), pltpu.roll(y[:, 128:], shift, axis=1)], axis=1)


def kernel(xT_hbm, wqkv_hbm, wo_hbm, w1_hbm, b1_hbm, w2_hbm, b2_hbm, out_hbm,
           xT, wqkv, wo, w1, b1, w2, b2,
           hT, xnT, tmpT, wqkvT, woT, u_acc, g,
           q_s, k_s, v_s, l1_s, p_s, o1c_s, o_s, outb, sems):
    lane256 = jax.lax.broadcasted_iota(jnp.int32, (8, C), 1) % 128

    def x_copy(c):
        return pltpu.make_async_copy(xT_hbm.at[:, pl.ds(c * C, C)], xT.at[:, pl.ds(c * C, C)], sems.at[c])

    def w1_copy(c):
        return pltpu.make_async_copy(w1_hbm.at[pl.ds(c * C, C), :], w1.at[pl.ds(c * C, C), :], sems.at[NC + c])

    def out_copy(c):
        return pltpu.make_async_copy(outb.at[:, pl.ds(c * C, C)], out_hbm.at[:, pl.ds(c * C, C)], sems.at[2 * NC + c])

    wqkv_copy = pltpu.make_async_copy(wqkv_hbm, wqkv, sems.at[3 * NC])
    wo_copy = pltpu.make_async_copy(wo_hbm, wo, sems.at[3 * NC + 1])
    b1_copy = pltpu.make_async_copy(b1_hbm, b1, sems.at[3 * NC + 2])
    b2_copy = pltpu.make_async_copy(b2_hbm, b2, sems.at[3 * NC + 3])
    w2_copy = pltpu.make_async_copy(w2_hbm, w2, sems.at[3 * NC + 4])

    def ln(c):
        for t in range(C // 128):
            cols = pl.ds(c * C + t * 128, 128)
            x = xT[:, cols].astype(F32)
            xn = _ln_cols(x)
            xnT[pl.ds(0, D), cols] = xn.astype(BF)
            h = _ln_cols(xn)
            hT[:, cols] = h.astype(BF)

    def u_mm(c):
        r = jnp.dot(hT[:, pl.ds(c * C, C)], w1[pl.ds(c * C, C), :], preferred_element_type=F32)
        if c == 0:
            u_acc[...] = r
        else:
            u_acc[...] += r

    def prep_wqkv():
        for kt in range(4):
            rows = 128 if kt < 3 else 64
            for ct in range(11):
                cols = 128 if ct < 10 else 64
                blk = wqkv[pl.ds(kt * 128, rows), pl.ds(ct * 128, cols)].astype(F32)
                tmpT[kt, pl.ds(ct * 128, cols), pl.ds(0, rows)] = blk.T
        lane = jax.lax.broadcasted_iota(jnp.int32, (16, 128), 1)
        for kt in range(4):
            for sec in range(3):
                for d in range(DH):
                    v = tmpT[kt, pl.ds(sec * D + d, H, stride=DH), :]
                    if kt == 3:
                        v = jnp.where(lane < 64, v, 0.0)
                    wqkvT[pl.ds(sec * D + d * H, H), pl.ds(kt * 128, 128)] = v.astype(BF)

    def prep_wo():
        for et in range(4):
            cols = 128 if et < 3 else 64
            tmpT[et, pl.ds(0, D), pl.ds(0, cols)] = wo[:, pl.ds(et * 128, cols)].astype(F32)
        for et in range(4):
            ecols = 128 if et < 3 else 64
            for ct in range(4):
                nd = 8 if ct < 3 else 4
                planes = [tmpT[et, pl.ds(ct * 8 + dd, H, stride=DH), :] for dd in range(nd)]
                if nd < 8:
                    planes.append(jnp.zeros(((8 - nd) * H, 128), F32))
                blk = jnp.concatenate(planes, axis=0)
                woT[pl.ds(et * 128, ecols), pl.ds(ct * 128, 128)] = blk.T[:ecols, :].astype(BF)

    def zero_pads():
        xnT[pl.ds(D, 64), :] = jnp.zeros((64, S), BF)
        o_s[pl.ds(D, 64), :] = jnp.zeros((64, S), F32)
        q_s[:, pl.ds(S, 128)] = jnp.zeros((D, 128), F32)
        k_s[:, pl.ds(0, 128)] = jnp.zeros((D, 128), F32)
        v_s[:, pl.ds(0, 128)] = jnp.zeros((D, 128), F32)
        for b in range(4):
            l1_s[b, :, pl.ds(0, 128)] = jnp.zeros((H, 128), F32)
            p_s[4 + b, :, pl.ds(S, 128)] = jnp.zeros((H, 128), F32)
        o1c_s[...] = jnp.zeros(o1c_s.shape, F32)

    def gelu_piece(j):
        cols = pl.ds(j * 128, 128)
        u = u_acc[:, cols] + b1row[:, j * 128:(j + 1) * 128]
        g[:, cols] = _gelu(u).astype(BF)

    def qkv_mm(c):
        cols = pl.ds(c * C, C)
        rhs = xnT[:, cols]
        q = jnp.dot(wqkvT[pl.ds(0, D), :], rhs, preferred_element_type=F32)
        q_s[:, cols] = q
        k = jnp.dot(wqkvT[pl.ds(D, D), :], rhs, preferred_element_type=F32)
        k_s[:, pl.ds(128 + c * C, C)] = k
        v = jnp.dot(wqkvT[pl.ds(2 * D, D), :], rhs, preferred_element_type=F32)
        v_s[:, pl.ds(128 + c * C, C)] = v

    def shr(xa, xb, n):
        if n == 0:
            return xb
        return _rot256(jnp.where(lane256 >= 128 - n, xa, xb), n)

    def shl(xa, xb, n):
        return _rot256(jnp.where(lane256 < n, xb, xa), 128 - n)

    def qk_softmax(c):
        t0 = c * C
        for hh in range(2):
            acc0 = [None] * 4
            acc1 = [None] * 4
            for d in range(DH):
                r = pl.ds(d * H + hh * 8, 8)
                qx = q_s[r, pl.ds(t0, C + 128)]
                kx = k_s[r, pl.ds(t0, C + 128)]
                q0 = qx[:, :C]
                q1 = shl(qx[:, :C], qx[:, 128:], 8)
                for b in range(4):
                    kb = shr(kx[:, :C], kx[:, 128:], 2 * b)
                    p0 = q0 * kb
                    p1 = q1 * kb
                    acc0[b] = p0 if d == 0 else acc0[b] + p0
                    acc1[b] = p1 if d == 0 else acc1[b] + p1
            hr = pl.ds(hh * 8, 8)
            logits = []
            for b in range(4):
                logits.append(acc0[b] * SCALE)
            for b in range(4):
                a1 = acc1[b] * SCALE
                prev = l1_s[b, hr, pl.ds(t0, 128)]
                l1_s[b, hr, pl.ds(128 + t0, C)] = a1
                xa = jnp.concatenate([prev, a1[:, :128]], axis=1)
                logits.append(shr(xa, a1, 8))
            if c == 0:
                pos = jax.lax.broadcasted_iota(jnp.int32, (8, C), 1)
                logits = [jnp.where(pos >= 2 * w, l, -1e9) for w, l in enumerate(logits)]
            m = logits[0]
            for w in range(1, W):
                m = jnp.maximum(m, logits[w])
            e = [jnp.exp(l - m) for l in logits]
            den = e[0]
            for w in range(1, W):
                den = den + e[w]
            inv = 1.0 / den
            for w in range(W):
                p_s[w, hr, pl.ds(t0, C)] = e[w] * inv

    def pv(c):
        t0 = c * C
        for hh in range(2):
            hr = pl.ds(hh * 8, 8)
            P = [p_s[w, hr, pl.ds(t0, C)] for w in range(4)]
            for b in range(4):
                px = p_s[4 + b, hr, pl.ds(t0, C + 128)]
                P.append(shl(px[:, :C], px[:, 128:], 8))
            for d in range(DH):
                r = pl.ds(d * H + hh * 8, 8)
                vx = v_s[r, pl.ds(t0, C + 128)]
                o0 = None
                o1 = None
                for b in range(4):
                    vb = shr(vx[:, :C], vx[:, 128:], 2 * b)
                    a = P[b] * vb
                    bb = P[4 + b] * vb
                    o0 = a if b == 0 else o0 + a
                    o1 = bb if b == 0 else o1 + bb
                prev = o1c_s[c, r, :]
                o1c_s[c + 1, r, :] = o1[:, 128:]
                xa = jnp.concatenate([prev, o1[:, :128]], axis=1)
                o_s[r, pl.ds(t0, C)] = o0 + shr(xa, o1, 8)

    def final(c):
        cols = pl.ds(c * C, C)
        y = jnp.dot(g[...], w2[:, cols], preferred_element_type=F32)
        a = jnp.dot(woT[...], o_s[:, cols].astype(BF), preferred_element_type=F32)
        res = y + a + b2row[:, c * C:(c + 1) * C] + xT[:, cols].astype(F32)
        outb[:, cols] = res.astype(BF)
        out_copy(c).start()

    x_copy(0).start()
    w1_copy(0).start()
    x_copy(1).start()
    w1_copy(1).start()
    for c in range(2, NC):
        x_copy(c).start()
        w1_copy(c).start()
    wqkv_copy.start()
    wo_copy.start()
    b1_copy.start()
    b2_copy.start()
    w2_copy.start()

    zero_pads()
    x_copy(0).wait()
    ln(0)
    for c in range(NC):
        if c + 1 < NC:
            x_copy(c + 1).wait()
            ln(c + 1)
        w1_copy(c).wait()
        u_mm(c)
        if c == 3:
            wqkv_copy.wait()
            prep_wqkv()
        if c == 5:
            wo_copy.wait()
            prep_wo()
    b1_copy.wait()
    b2_copy.wait()
    b1row = b1[...].astype(F32).reshape(1, F)
    b2row = b2[...].astype(F32).reshape(1, S)

    gelu_sched = [[0, 1], [2, 3], [4, 5], [6, 7], [8, 9], [10, 11], [12], [13]]
    for c in range(NC):
        qkv_mm(c)
        for j in gelu_sched[c]:
            gelu_piece(j)
        if c >= 2:
            qk_softmax(c - 2)
        if c >= 4:
            pv(c - 4)
    w2_copy.wait()
    qk_softmax(NC - 2)
    qk_softmax(NC - 1)
    for c in range(NC):
        if c + 4 < NC:
            pv(c + 4)
        final(c)
    for c in range(NC):
        out_copy(c).wait()


def _call(xT, wqkv, wo, w1, b1, w2, b2):
    any_spec = pl.BlockSpec(memory_space=pl.ANY)
    scratch = [
        pltpu.VMEM((D, S), BF), pltpu.VMEM((D, 3 * D), BF), pltpu.VMEM((D, D), BF),
        pltpu.VMEM((S, F), BF), pltpu.VMEM((F,), BF), pltpu.VMEM((F, S), BF), pltpu.VMEM((S,), BF),
        pltpu.VMEM((D, S), BF),
        pltpu.VMEM((512, S), BF),
        pltpu.VMEM((4, 1408, 128), F32),
        pltpu.VMEM((3 * D, 512), BF),
        pltpu.VMEM((D, 512), BF),
        pltpu.VMEM((D, F), F32),
        pltpu.VMEM((D, F), BF),
        pltpu.VMEM((D, S + 128), F32),
        pltpu.VMEM((D, S + 128), F32),
        pltpu.VMEM((D, S + 128), F32),
        pltpu.VMEM((4, H, S + 128), F32),
        pltpu.VMEM((W, H, S + 128), F32),
        pltpu.VMEM((NC + 1, D, 128), F32),
        pltpu.VMEM((512, S), F32),
        pltpu.VMEM((D, S), BF),
        pltpu.SemaphoreType.DMA((3 * NC + 5,)),
    ]
    return pl.pallas_call(
        kernel,
        out_shape=jax.ShapeDtypeStruct((D, S), BF),
        in_specs=[any_spec] * 7,
        out_specs=any_spec,
        scratch_shapes=scratch,
        compiler_params=pltpu.CompilerParams(vmem_limit_bytes=110 * 1024 * 1024),
    )(xT, wqkv, wo, w1, b1, w2, b2)


@jax.jit
def pallas_parallel_sum__sliding_local_dilated__mixer_token_mlp__prompt_kernel(A_x, A_wqkv, A_wo, B_x, B_w1, B_b1, B_w2, B_b2):
    outT = _call(A_x[0].T, A_wqkv, A_wo, B_w1, B_b1, B_w2, B_b2)
    return outT.T[None]
```

```python
import jax
import jax.numpy as jnp
import jax.experimental.pallas as pl
import jax.experimental.pallas.tpu as pltpu

S, D, H, DH, F = 2048, 448, 16, 28, 1792
W = 8
C = 256
NC = S // C
KA = 1024
NG = 256
NJ = F // NG
EPS = 1e-5
SCALE = DH ** -0.5
BF, F32, U32 = jnp.bfloat16, jnp.float32, jnp.uint32
NTOK = 4
LN_RB = 32


def _gelu(x):
    c0 = 0.7978845608028654
    inner = c0 * (x + 0.044715 * (x * x * x))
    return 0.5 * x * (1.0 + jnp.tanh(inner))


def _rot256(y, shift):
    return jnp.concatenate(
        [pltpu.roll(y[:, :128], shift, axis=1), pltpu.roll(y[:, 128:], shift, axis=1)], axis=1)


def _tok(v):
    return (pltpu.bitcast(v[0:8, 0:128], U32) >> 31) >> 1


def _gate_f32(x, tk):
    if tk is None:
        return x
    t = jnp.tile(tk, (x.shape[0] // 8, x.shape[1] // 128))
    return jax.lax.bitcast_convert_type(pltpu.bitcast(x, U32) | t, F32)


def _gate_words(xb, tk):
    wd = pltpu.bitcast(xb, U32)
    if tk is None:
        return wd
    return wd | jnp.tile(tk, (wd.shape[0] // 8, wd.shape[1] // 128))


def kernel(xT_hbm, wqkv_hbm, wo_hbm, w1_hbm, b1_hbm, w2_hbm, b2_hbm, out_hbm,
           xT, wqkv, wo, w1, b1, w2, b2,
           hT, xnT, tmpT, tmpU, wqkvT, woT, g,
           q_s, k_s, v_s, l1_s, p_s, o1c_s, o_s, outb, sems):
    lane256 = jax.lax.broadcasted_iota(jnp.int32, (8, C), 1) % 128

    groups = {}

    def add(gname, src, dst):
        if gname not in groups:
            groups[gname] = (len(groups), [])
        idx, lst = groups[gname]
        lst.append(pltpu.make_async_copy(src, dst, sems.at[idx]))

    def add_x(gname, t0, t1):
        for a0 in range(t0, t1, 128):
            add(gname, xT_hbm.at[:, pl.ds(a0, 128)], xT.at[a0 // 128])

    def add_w1(gname, r0, r1, c0, c1, step):
        for j in range(c0 // 128, c1 // 128):
            for a0 in range(r0, r1, step):
                add(gname, w1_hbm.at[pl.ds(a0, step), pl.ds(j * 128, 128)], w1.at[j, pl.ds(a0, step), :])

    def add_rows(gname, src, dst, step):
        for a0 in range(0, src.shape[0], step):
            add(gname, src.at[pl.ds(a0, step), :], dst.at[pl.ds(a0, step), :])

    def start(gname):
        for cp in groups[gname][1]:
            cp.start()

    def wait(gname):
        for cp in groups[gname][1]:
            cp.wait()

    def add_cols(gname, src_, dst, c0, c1, rstep):
        for a0 in range(0, src_.shape[0], rstep):
            add(gname, src_.at[pl.ds(a0, rstep), pl.ds(c0, c1 - c0)], dst.at[pl.ds(a0, rstep), pl.ds(c0, c1 - c0)])

    add_x("x0", 0, 256)
    add_x("x1", 256, 512)
    add_cols("wq", wqkv_hbm, wqkv, 0, 512, 224)
    add_cols("wkv", wqkv_hbm, wqkv, 512, 896, 224); add_cols("wkv", wqkv_hbm, wqkv, 896, 3 * D, 224)
    add_x("wkv", 512, 768)
    add_x("x2", 768, S)
    for j in range(0, 4):
        add_w1("w1a", 0, S, j * NG, (j + 1) * NG, 1024)
    add("w1a", b1_hbm, b1)
    for j in range(4, NJ):
        add_w1("w1b", 0, S, j * NG, (j + 1) * NG, 1024)
    add_rows("w1b", wo_hbm, wo, 224)
    add("w2", b2_hbm, b2)
    for j in range(S // 128):
        for a0 in range(0, F, 896):
            add("w2", w2_hbm.at[pl.ds(a0, 896), pl.ds(j * 128, 128)], w2.at[j, pl.ds(a0, 896), :])
    n_in = len(groups)

    def out_copies(c):
        return [pltpu.make_async_copy(outb.at[2 * c + i], out_hbm.at[:, pl.ds((2 * c + i) * 128, 128)], sems.at[n_in + c])
                for i in range(2)]

    def cat(ref, tiles, r0=0, nr=None):
        nr = ref.shape[1] - r0 if nr is None else nr
        words = ref.bitcast(U32)
        return jnp.concatenate([pltpu.bitcast(words[t, pl.ds(r0 // 2, nr // 2), :], BF) for t in tiles], axis=1)

    def release(r, pieces, ntok=NTOK):
        n = len(pieces)
        done = 0
        for q in range(ntok):
            upto = (n * (q + 1)) // ntok
            if done < upto:
                tk = _tok(r[q * (r.shape[0] // ntok):, :]) if r is not None else None
                while done < upto:
                    pieces[done](tk)
                    done += 1

    def split(lst, n):
        return [lst[(len(lst) * i) // n:(len(lst) * (i + 1)) // n] for i in range(n)]

    def ln_pieces(t):
        RB = LN_RB
        st = {}

        def p1(r0):
            def step(tk):
                wd = _gate_words(xT[t, pl.ds(r0, RB), :], tk)
                lo = jax.lax.bitcast_convert_type(wd << 16, F32)
                hi = jax.lax.bitcast_convert_type(wd & U32(0xFFFF0000), F32)
                if r0 == 0:
                    st["c"] = jnp.broadcast_to(lo[0:1, :], (RB // 2, 128))
                a = lo - st["c"]
                b = hi - st["c"]
                p = a + b
                q = a * a + b * b
                st["s1"] = p if r0 == 0 else st["s1"] + p
                st["s2"] = q if r0 == 0 else st["s2"] + q
            return step

        def stats(tk):
            s1 = jnp.sum(st["s1"], axis=0, keepdims=True) * (1.0 / D)
            s2 = jnp.sum(st["s2"], axis=0, keepdims=True) * (1.0 / D)
            st["m"] = st["c"][0:1] + s1
            v = s2 - s1 * s1
            r = jax.lax.rsqrt(v + EPS)
            st["r"] = r
            st["rr"] = r * jax.lax.rsqrt(v * (r * r) + EPS)

        def p2(r0):
            def step(tk):
                wd = _gate_words(xT[t, pl.ds(r0, RB), :], tk)
                xc = pltpu.bitcast(wd, BF).astype(F32) - st["m"]
                xnT[t, pl.ds(r0, RB), :] = (xc * st["r"]).astype(BF)
                hT[t, pl.ds(r0, RB), :] = (xc * st["rr"]).astype(BF)
            return step

        return [p1(r0) for r0 in range(0, D, RB)] + [stats] + [p2(r0) for r0 in range(0, D, RB)]

    def ln_steps(t0, t1):
        return [s for t in range(t0, t1) for s in ln_pieces(t)]

    def h_cols(t0, t1):
        return cat(hT, range(t0 // 128, t1 // 128))

    def u_group(j, pieces=()):
        cols = pl.ds(j * NG, NG)
        parts = split(list(pieces), 4)
        acc = None
        for i in range(4):
            r = jnp.dot(h_cols(i * 512, (i + 1) * 512), cat(w1, (2 * j, 2 * j + 1), i * 512, 512), preferred_element_type=F32)
            release(r, parts[i])
            acc = r if acc is None else acc + r
        act = _gelu(acc + b1row[:, j * NG:(j + 1) * NG]).astype(BF)
        g[2 * j] = act[:, :128]
        g[2 * j + 1] = act[:, 128:]

    def prep_wqkv_pieces(sec):
        def tr(kt, ct):
            rows = 128 if kt < 3 else 64
            cols = 128 if ct < 10 else 64

            def step(tk):
                blk = wqkv[pl.ds(kt * 128, rows), pl.ds(ct * 128, cols)]
                if tk is not None and cols == 128:
                    blk = pltpu.bitcast(_gate_words(blk, tk), BF)
                tmpU[kt, pl.ds(ct * 64, cols // 2), pl.ds(0, rows)] = pltpu.bitcast(blk.T, U32)
            return step

        lane = jax.lax.broadcasted_iota(jnp.int32, (16, 128), 1)

        def ga(kt, d0):
            def step(tk):
                for d in range(d0, d0 + 4, 2):
                    wd = tmpU[kt, pl.ds((sec * D + d) // 2, H, stride=DH // 2), :]
                    if tk is not None:
                        wd = wd | jnp.tile(tk, (2, 1))
                    lo = jax.lax.bitcast_convert_type(wd << 16, F32)
                    hi = jax.lax.bitcast_convert_type(wd & U32(0xFFFF0000), F32)
                    if kt == 3:
                        lo = jnp.where(lane < 64, lo, 0.0)
                        hi = jnp.where(lane < 64, hi, 0.0)
                    wqkvT[kt, pl.ds(sec * D + d * H, H), :] = lo.astype(BF)
                    wqkvT[kt, pl.ds(sec * D + (d + 1) * H, H), :] = hi.astype(BF)
            return step

        c_lo = (sec * D) // 128
        c_hi = (sec * D + D - 1) // 128
        if sec > 0:
            c_lo += 1 if sec * D % 128 else 0
        a = [tr(kt, ct) for ct in range(c_lo, c_hi + 1) for kt in range(4)]
        b = [ga(kt, d0) for kt in range(4) for d0 in range(0, DH, 4)]
        return a + b

    def prep_wo_pieces():
        def cp(et, r0):
            cols = 128 if et < 3 else 64

            def step(tk):
                blk = wo[pl.ds(r0, 112), pl.ds(et * 128, cols)]
                if tk is not None and cols == 128:
                    blk = pltpu.bitcast(_gate_words(blk, tk), BF)
                tmpT[et, pl.ds(r0, 112), pl.ds(0, cols)] = blk.astype(F32)
            return step

        def ga(et, ct):
            ecols = 128 if et < 3 else 64
            nd = 8 if ct < 3 else 4

            def step(tk):
                planes = [_gate_f32(tmpT[et, pl.ds(ct * 8 + dd, H, stride=DH), :], tk) for dd in range(nd)]
                if nd < 8:
                    planes.append(jnp.zeros(((8 - nd) * H, 128), F32))
                blk = jnp.concatenate(planes, axis=0)
                woT[ct, pl.ds(et * 128, ecols), :] = blk.T[:ecols, :].astype(BF)
            return step

        a = [cp(et, r0) for et in range(4) for r0 in range(0, D, 112)]
        b = [ga(et, ct) for et in range(4) for ct in range(4)]
        return a + b

    def zero_pads():
        xnT[:, pl.ds(D, 64), :] = jnp.zeros((S // 128, 64, 128), BF)
        o_s[pl.ds(D, 64), :] = jnp.zeros((64, S), F32)
        q_s[:, pl.ds(S, 128)] = jnp.zeros((D, 128), F32)
        k_s[:, pl.ds(0, 128)] = jnp.zeros((D, 128), F32)
        v_s[:, pl.ds(0, 128)] = jnp.zeros((D, 128), F32)
        for b in range(4):
            l1_s[b, :, pl.ds(0, 128)] = jnp.zeros((H, 128), F32)
            p_s[4 + b, :, pl.ds(S, 128)] = jnp.zeros((H, 128), F32)
        o1c_s[0] = jnp.zeros((D, 128), F32)

    def qkv_dot(c, sec, pieces):
        rhs = cat(xnT, (2 * c, 2 * c + 1))
        r = jnp.dot(cat(wqkvT, range(4), sec * D, D), rhs, preferred_element_type=F32)
        if sec == 0:
            q_s[:, pl.ds(c * C, C)] = r
        elif sec == 1:
            k_s[:, pl.ds(128 + c * C, C)] = r
        else:
            v_s[:, pl.ds(128 + c * C, C)] = r
        release(r, pieces)

    def shr(xa, xb, n):
        if n == 0:
            return xb
        return _rot256(jnp.where(lane256 >= 128 - n, xa, xb), n)

    def shl(xa, xb, n):
        return _rot256(jnp.where(lane256 < n, xb, xa), 128 - n)

    def qk_pieces(c):
        t0 = c * C
        st = {}

        def qk(hh, d):
            def step(tk):
                r = pl.ds(d * H + hh * 8, 8)
                qx = _gate_f32(q_s[r, pl.ds(t0, C + 128)], tk)
                kx = _gate_f32(k_s[r, pl.ds(t0, C + 128)], tk)
                q0 = qx[:, :C]
                q1 = shl(qx[:, :C], qx[:, 128:], 8)
                for b in range(4):
                    kb = shr(kx[:, :C], kx[:, 128:], 2 * b)
                    p0 = q0 * kb
                    p1 = q1 * kb
                    st[0, b] = p0 if d == 0 else st[0, b] + p0
                    st[1, b] = p1 if d == 0 else st[1, b] + p1
            return step

        def softmax(hh):
            def step(tk):
                hr = pl.ds(hh * 8, 8)
                logits = [st[0, b] * SCALE for b in range(4)]
                for b in range(4):
                    a1 = st[1, b] * SCALE
                    prev = l1_s[b, hr, pl.ds(t0, 128)]
                    l1_s[b, hr, pl.ds(128 + t0, C)] = a1
                    xa = jnp.concatenate([prev, a1[:, :128]], axis=1)
                    logits.append(shr(xa, a1, 8))
                if c == 0:
                    pos = jax.lax.broadcasted_iota(jnp.int32, (8, C), 1)
                    logits = [jnp.where(pos >= 2 * w, l, -1e9) for w, l in enumerate(logits)]
                m = logits[0]
                for w in range(1, W):
                    m = jnp.maximum(m, logits[w])
                e = [jnp.exp(l - m) for l in logits]
                den = e[0]
                for w in range(1, W):
                    den = den + e[w]
                inv = 1.0 / den
                for w in range(W):
                    p_s[w, hr, pl.ds(t0, C)] = e[w] * inv
            return step

        out = []
        for hh in range(2):
            out += [qk(hh, d) for d in range(DH)] + [softmax(hh)]
        return out

    def pv_pieces(c):
        t0 = c * C
        st = {}

        def load_p(hh):
            def step(tk):
                hr = pl.ds(hh * 8, 8)
                P = [p_s[w, hr, pl.ds(t0, C)] for w in range(4)]
                for b in range(4):
                    px = p_s[4 + b, hr, pl.ds(t0, C + 128)]
                    P.append(shl(px[:, :C], px[:, 128:], 8))
                st["P"] = P
            return step

        def pv(hh, d):
            def step(tk):
                P = st["P"]
                r = pl.ds(d * H + hh * 8, 8)
                vx = _gate_f32(v_s[r, pl.ds(t0, C + 128)], tk)
                o0 = None
                o1 = None
                for b in range(4):
                    vb = shr(vx[:, :C], vx[:, 128:], 2 * b)
                    a = P[b] * vb
                    bb = P[4 + b] * vb
                    o0 = a if b == 0 else o0 + a
                    o1 = bb if b == 0 else o1 + bb
                prev = o1c_s[c, r, :]
                if c + 1 < NC:
                    o1c_s[c + 1, r, :] = o1[:, 128:]
                xa = jnp.concatenate([prev, o1[:, :128]], axis=1)
                o_s[r, pl.ds(t0, C)] = o0 + shr(xa, o1, 8)
            return step

        out = []
        for hh in range(2):
            out += [load_p(hh)] + [pv(hh, d) for d in range(DH)]
        return out

    def final(c, pieces):
        cols = pl.ds(c * C, C)
        parts = split(pieces, 5)
        acc = None
        for i, (k0, k1) in enumerate(((0, 512), (512, 1024), (1024, 1536), (1536, F))):
            r = jnp.dot(cat(g, range(k0 // 128, k1 // 128)), cat(w2, (2 * c, 2 * c + 1), k0, k1 - k0),
                        preferred_element_type=F32)
            release(r, parts[i])
            acc = r if acc is None else acc + r
        a = jnp.dot(cat(woT, range(4)), o_s[:, cols].astype(BF), preferred_element_type=F32)
        release(a, parts[4])
        xr = jnp.concatenate([xT[2 * c], xT[2 * c + 1]], axis=1).astype(F32)
        res = (acc + a) + b2row[:, c * C:(c + 1) * C] + xr
        resb = res.astype(BF)
        outb[2 * c] = resb[:, :128]
        outb[2 * c + 1] = resb[:, 128:]
        for cp in out_copies(c):
            cp.start()

    start("x0"); start("x1"); start("wq")
    zero_pads()
    wait("x0")
    start("wkv")
    release(None, ln_steps(0, 2))
    wait("x1")
    release(None, ln_steps(2, 4))
    wait("wq")
    start("x2")
    release(None, prep_wqkv_pieces(0))
    qkv_dot(0, 0, [])
    qkv_dot(1, 0, [])
    wait("wkv")
    start("w1a")
    release(None, prep_wqkv_pieces(1))
    pv_ = prep_wqkv_pieces(2)
    l45 = ln_steps(4, 6)
    qkv_dot(0, 1, pv_[:len(pv_) // 2])
    qkv_dot(1, 1, pv_[len(pv_) // 2:])
    qkv_dot(0, 2, l45[:29])
    qkv_dot(1, 2, l45[29:])
    wait("x2")
    start("w1b"); start("w2")
    att = {(c, s): [] for c in range(NC) for s in range(3)}
    for c in range(2, NC - 1):
        a, b, d_ = split(ln_steps(2 * c + 2, 2 * c + 4), 3)
        att[c, 0] += a
        att[c, 1] += b
        att[c, 2] += d_
    a, b, d_ = split(qk_pieces(0), 3)
    att[7, 0] += a
    att[7, 1] += b
    att[7, 2] += d_
    for c in range(2, NC):
        for s in range(3):
            qkv_dot(c, s, att[c, s])
    wait("w1a")
    b1row = b1[...].astype(F32).reshape(1, F)
    u_group(0, qk_pieces(1))
    u_group(1, qk_pieces(2))
    u_group(2, qk_pieces(3))
    u_group(3, qk_pieces(4))
    wait("w1b")
    u_group(4, qk_pieces(5) + prep_wo_pieces())
    u_group(5, qk_pieces(6) + pv_pieces(0)[:29])
    u_group(6, qk_pieces(7) + pv_pieces(0)[29:])
    wait("w2")
    b2row = b2[...].astype(F32).reshape(1, S)
    fin = {c: [] for c in range(NC)}
    for c in range(NC - 1):
        fin[c] += pv_pieces(c + 1)
    for c in range(NC):
        final(c, fin[c])
    for c in range(NC):
        for cp in out_copies(c):
            cp.wait()


def _call(xT, wqkv, wo, w1, b1, w2, b2):
    any_spec = pl.BlockSpec(memory_space=pl.ANY)
    scratch = [
        pltpu.VMEM((S // 128, D, 128), BF), pltpu.VMEM((D, 3 * D), BF), pltpu.VMEM((D, D), BF),
        pltpu.VMEM((F // 128, S, 128), BF), pltpu.VMEM((F,), BF), pltpu.VMEM((S // 128, F, 128), BF), pltpu.VMEM((S,), BF),
        pltpu.VMEM((S // 128, D, 128), BF),
        pltpu.VMEM((S // 128, 512, 128), BF),
        pltpu.VMEM((4, D, 128), F32),
        pltpu.VMEM((4, 672, 128), U32),
        pltpu.VMEM((4, 3 * D, 128), BF),
        pltpu.VMEM((4, D, 128), BF),
        pltpu.VMEM((F // 128, D, 128), BF),
        pltpu.VMEM((D, S + 128), F32),
        pltpu.VMEM((D, S + 128), F32),
        pltpu.VMEM((D, S + 128), F32),
        pltpu.VMEM((4, H, S + 128), F32),
        pltpu.VMEM((W, H, S + 128), F32),
        pltpu.VMEM((NC, D, 128), F32),
        pltpu.VMEM((512, S), F32),
        pltpu.VMEM((S // 128, D, 128), BF),
        pltpu.SemaphoreType.DMA((8 + NC,)),
    ]
    return pl.pallas_call(
        kernel,
        out_shape=jax.ShapeDtypeStruct((D, S), BF),
        in_specs=[any_spec] * 7,
        out_specs=any_spec,
        scratch_shapes=scratch,
        compiler_params=pltpu.CompilerParams(vmem_limit_bytes=110 * 1024 * 1024),
    )(xT, wqkv, wo, w1, b1, w2, b2)


@jax.jit
def pallas_parallel_sum__sliding_local_dilated__mixer_token_mlp__prompt_kernel(A_x, A_wqkv, A_wo, B_x, B_w1, B_b1, B_w2, B_b2):
    outT = _call(A_x[0].T, A_wqkv, A_wo, B_w1, B_b1, B_w2, B_b2)
    return outT.T[None]
```

```python
import jax
import jax.numpy as jnp
import jax.experimental.pallas as pl
import jax.experimental.pallas.tpu as pltpu

S, D, H, DH, F = 2048, 448, 16, 28, 1792
W = 8
C = 256
NC = S // C
NG = 256
NJ = F // NG
EPS = 1e-5
SCALE = DH ** -0.5
BF, F32, U32 = jnp.bfloat16, jnp.float32, jnp.uint32
NTOK = 8
LN_RB = 32


def _gelu(x):
    c0 = 0.7978845608028654
    inner = c0 * (x + 0.044715 * (x * x * x))
    return 0.5 * x * (1.0 + jnp.tanh(inner))


def _rot256(y, shift):
    return jnp.concatenate(
        [pltpu.roll(y[:, :128], shift, axis=1), pltpu.roll(y[:, 128:], shift, axis=1)], axis=1)


def _tok(v):
    return (pltpu.bitcast(v[0:8, 0:128], U32) >> 31) >> 1


def _gate_f32(x, tk):
    if tk is None:
        return x
    t = jnp.tile(tk, (x.shape[0] // 8, x.shape[1] // 128))
    return jax.lax.bitcast_convert_type(pltpu.bitcast(x, U32) | t, F32)


def _gate(wd, tk):
    if tk is None:
        return wd
    return wd | jnp.tile(tk, (wd.shape[0] // 8, wd.shape[1] // 128))


def _gate_mid(x, tk):
    if tk is None:
        return x
    return jnp.concatenate([x[:, :128], _gate_f32(x[:, 128:256], tk), x[:, 256:]], axis=1)


def _gate_words(xb, tk):
    wd = pltpu.bitcast(xb, U32)
    if tk is None:
        return wd
    return wd | jnp.tile(tk, (wd.shape[0] // 8, wd.shape[1] // 128))


def kernel(xT_hbm, wqkv_hbm, wo_hbm, w1_hbm, b1_hbm, w2_hbm, b2_hbm, out_hbm,
           xT, wqkv, wo, w1, b1, w2, b2,
           hT, xnT, tmpT, tmpU, wqkvT, woT, g,
           q_s, k_s, v_s, l1_s, p_s, o1c_s, o_s, outb, sems):
    lane256 = jax.lax.broadcasted_iota(jnp.int32, (8, C), 1) % 128

    groups = {}

    def add(gname, src, dst):
        if gname not in groups:
            groups[gname] = (len(groups), [])
        idx, lst = groups[gname]
        lst.append(pltpu.make_async_copy(src, dst, sems.at[idx]))

    def add_x(gname, t0, t1):
        for a0 in range(t0, t1, 128):
            add(gname, xT_hbm.at[:, pl.ds(a0, 128)], xT.at[a0 // 128])

    def add_w1(gname, r0, r1, c0, c1, step):
        for j in range(c0 // 128, c1 // 128):
            for a0 in range(r0, r1, step):
                add(gname, w1_hbm.at[pl.ds(a0, step), pl.ds(j * 128, 128)], w1.at[j, pl.ds(a0, step), :])

    def add_rows(gname, src, dst, step):
        for a0 in range(0, src.shape[0], step):
            add(gname, src.at[pl.ds(a0, step), :], dst.at[pl.ds(a0, step), :])

    def start(gname):
        for cp in groups[gname][1]:
            cp.start()

    def wait(gname):
        for cp in groups[gname][1]:
            cp.wait()

    def add_cols(gname, src_, dst, c0, c1, rstep):
        for a0 in range(0, src_.shape[0], rstep):
            add(gname, src_.at[pl.ds(a0, rstep), pl.ds(c0, c1 - c0)], dst.at[pl.ds(a0, rstep), pl.ds(c0, c1 - c0)])

    add_cols("wq", wqkv_hbm, wqkv, 0, 512, 224)
    add_x("x0", 0, 256)
    add_x("x1", 256, 512)
    add_cols("wk", wqkv_hbm, wqkv, 512, 896, 224)
    add_cols("wv", wqkv_hbm, wqkv, 896, 3 * D, 224)
    add_x("wv", 512, 768)
    add_x("x2", 768, S)
    for j in range(0, 4):
        add_w1("w1a", 0, S, j * NG, (j + 1) * NG, 1024)
    add("w1a", b1_hbm, b1)
    for j in range(4, NJ):
        add_w1("w1b", 0, S, j * NG, (j + 1) * NG, 1024)
    add_rows("w1b", wo_hbm, wo, 224)
    add("w2", b2_hbm, b2)
    for j in range(S // 128):
        for a0 in range(0, F, 896):
            add("w2", w2_hbm.at[pl.ds(a0, 896), pl.ds(j * 128, 128)], w2.at[j, pl.ds(a0, 896), :])
    n_in = len(groups)

    def out_blocks(c):
        return [(0, D)] if c + 1 < NC else [(r0, 112) for r0 in range(0, D, 112)]

    def out_copies(c, r0, nr):
        return [pltpu.make_async_copy(outb.at[2 * c + i, pl.ds(r0, nr), :],
                                      out_hbm.at[pl.ds(r0, nr), pl.ds((2 * c + i) * 128, 128)], sems.at[n_in + c])
                for i in range(2)]

    def cat(ref, tiles, r0=0, nr=None):
        nr = ref.shape[1] - r0 if nr is None else nr
        words = ref.bitcast(U32)
        return jnp.concatenate([pltpu.bitcast(words[t, pl.ds(r0 // 2, nr // 2), :], BF) for t in tiles], axis=1)

    def release(r, pieces, ntok=NTOK):
        n = len(pieces)
        done = 0
        for q in range(ntok):
            upto = (n * (q + 1)) // ntok
            if done < upto:
                tk = _tok(r[q * (r.shape[0] // ntok):, :]) if r is not None else None
                while done < upto:
                    pieces[done](tk)
                    done += 1

    def split(lst, n):
        return [lst[(len(lst) * i) // n:(len(lst) * (i + 1)) // n] for i in range(n)]

    xw = xT.bitcast(U32)
    def ln_pieces(t):
        RB = LN_RB
        st = {}

        def p1(r0):
            def step(tk):
                wd = _gate(xw[t, pl.ds(r0 // 2, RB // 2), :], tk)
                lo = jax.lax.bitcast_convert_type(wd << 16, F32)
                hi = jax.lax.bitcast_convert_type(wd & U32(0xFFFF0000), F32)
                if r0 == 0:
                    st["c"] = jnp.broadcast_to(lo[0:1, :], (RB // 2, 128))
                a = lo - st["c"]
                b = hi - st["c"]
                p = a + b
                q = a * a + b * b
                st["s1"] = p if r0 == 0 else st["s1"] + p
                st["s2"] = q if r0 == 0 else st["s2"] + q
            return step

        def stats(tk):
            s1 = jnp.sum(st["s1"], axis=0, keepdims=True) * (1.0 / D)
            s2 = jnp.sum(st["s2"], axis=0, keepdims=True) * (1.0 / D)
            st["m"] = st["c"][0:1] + s1
            v = s2 - s1 * s1
            r = jax.lax.rsqrt(v + EPS)
            st["r"] = r
            st["rr"] = r * jax.lax.rsqrt(v * (r * r) + EPS)

        def p2(r0):
            def step(tk):
                wd = _gate(xw[t, pl.ds(r0 // 2, RB // 2), :], tk)
                xc = pltpu.bitcast(wd, BF).astype(F32) - st["m"]
                xnT[t, pl.ds(r0, RB), :] = (xc * st["r"]).astype(BF)
                hT[t, pl.ds(r0, RB), :] = (xc * st["rr"]).astype(BF)
            return step

        return [p1(r0) for r0 in range(0, D, RB)] + [stats] + [p2(r0) for r0 in range(0, D, RB)]

    def ln_steps(t0, t1):
        return [s for t in range(t0, t1) for s in ln_pieces(t)]

    def h_cols(t0, t1):
        return cat(hT, range(t0 // 128, t1 // 128))

    def u_group(j, pieces=(), mid=None):
        parts = split(list(pieces), 4)
        acc = None
        for i in range(4):
            if i == 2 and mid is not None:
                mid()
            r = jnp.dot(h_cols(i * 512, (i + 1) * 512), cat(w1, (2 * j, 2 * j + 1), i * 512, 512), preferred_element_type=F32)
            release(r, parts[i])
            acc = r if acc is None else acc + r
        act = _gelu(acc + b1row[:, j * NG:(j + 1) * NG]).astype(BF)
        g[2 * j] = act[:, :128]
        g[2 * j + 1] = act[:, 128:]

    def prep_wqkv_pieces(sec):
        def tr(kt, ct):
            rows = 128 if kt < 3 else 64
            cols = 128 if ct < 10 else 64

            def step(tk):
                blk = wqkv[pl.ds(kt * 128, rows), pl.ds(ct * 128, cols)]
                if tk is not None and cols == 128:
                    blk = pltpu.bitcast(_gate_words(blk, tk), BF)
                tmpU[kt, pl.ds(ct * 64, cols // 2), pl.ds(0, rows)] = pltpu.bitcast(blk.T, U32)
            return step

        def ga(kt, d0):
            def step(tk):
                for d in range(d0, d0 + 4, 2):
                    wd = tmpU[kt, pl.ds((sec * D + d) // 2, H, stride=DH // 2), :]
                    if tk is not None:
                        wd = wd | jnp.tile(tk, (2, 1))
                    lo = jax.lax.bitcast_convert_type(wd << 16, F32)
                    hi = jax.lax.bitcast_convert_type(wd & U32(0xFFFF0000), F32)
                    wqkvT[kt, pl.ds(sec * D + d * H, H), :] = lo.astype(BF)
                    wqkvT[kt, pl.ds(sec * D + (d + 1) * H, H), :] = hi.astype(BF)
            return step

        c_lo = (sec * D) // 128
        c_hi = (sec * D + D - 1) // 128
        if sec > 0:
            c_lo += 1 if sec * D % 128 else 0
        a = [tr(kt, ct) for ct in range(c_lo, c_hi + 1) for kt in range(4)]
        b = [ga(kt, d0) for kt in range(4) for d0 in range(0, DH, 4)]
        return a + b

    def prep_wo_pieces():
        def cp(et, r0):
            cols = 128 if et < 3 else 64

            def step(tk):
                blk = wo[pl.ds(r0, 112), pl.ds(et * 128, cols)]
                if tk is not None and cols == 128:
                    blk = pltpu.bitcast(_gate_words(blk, tk), BF)
                tmpT[et, pl.ds(r0, 112), pl.ds(0, cols)] = blk.astype(F32)
            return step

        def ga(et, ct):
            ecols = 128 if et < 3 else 64
            nd = 8 if ct < 3 else 4

            def step(tk):
                planes = [_gate_f32(tmpT[et, pl.ds(ct * 8 + dd, H, stride=DH), :], tk) for dd in range(nd)]
                if nd < 8:
                    planes.append(jnp.zeros(((8 - nd) * H, 128), F32))
                blk = jnp.concatenate(planes, axis=0)
                woT[ct, pl.ds(et * 128, ecols), :] = blk.T[:ecols, :].astype(BF)
            return step

        a = [cp(et, r0) for et in range(4) for r0 in range(0, D, 112)]
        b = [ga(et, ct) for et in range(4) for ct in range(4)]
        return a + b

    def zero_pads():
        xnT[:, pl.ds(D, 64), :] = jnp.zeros((S // 128, 64, 128), BF)
        o_s[pl.ds(D, 64), :] = jnp.zeros((64, S), F32)
        q_s[:, pl.ds(S, 128)] = jnp.zeros((D, 128), F32)
        k_s[:, pl.ds(0, 128)] = jnp.zeros((D, 128), F32)
        v_s[:, pl.ds(0, 128)] = jnp.zeros((D, 128), F32)
        for b in range(4):
            l1_s[b, :, pl.ds(0, 128)] = jnp.zeros((H, 128), F32)
            p_s[4 + b, :, pl.ds(S, 128)] = jnp.zeros((H, 128), F32)
        o1c_s[0] = jnp.zeros((D, 128), F32)
        tmpU[3] = jnp.zeros((672, 128), U32)
        tmpT[3] = jnp.zeros((D, 128), F32)

    def qkv_dot(c, sec, pieces, r0=0, nr=D):
        rhs = cat(xnT, (2 * c, 2 * c + 1))
        r = jnp.dot(cat(wqkvT, range(4), sec * D + r0, nr), rhs, preferred_element_type=F32)
        dst, off = ((q_s, 0), (k_s, 128), (v_s, 128))[sec]
        dst[pl.ds(r0, nr), pl.ds(off + c * C, C)] = r
        release(r, pieces)

    def shr(xa, xb, n):
        if n == 0:
            return xb
        return _rot256(jnp.where(lane256 >= 128 - n, xa, xb), n)

    def shl(xa, xb, n):
        return _rot256(jnp.where(lane256 < n, xb, xa), 128 - n)

    def qk_pieces(c):
        t0 = c * C
        st = {}

        def qk(hh, d):
            def step(tk):
                r = pl.ds(d * H + hh * 8, 8)
                qx = _gate_mid(q_s[r, pl.ds(t0, C + 128)], tk)
                kx = _gate_mid(k_s[r, pl.ds(t0, C + 128)], tk)
                q0 = qx[:, :C]
                q1 = shl(qx[:, :C], qx[:, 128:], 8)
                for b in range(4):
                    kb = shr(kx[:, :C], kx[:, 128:], 2 * b)
                    p0 = q0 * kb
                    p1 = q1 * kb
                    st[0, b] = p0 if d == 0 else st[0, b] + p0
                    st[1, b] = p1 if d == 0 else st[1, b] + p1
            return step

        def softmax(hh):
            def step(tk):
                hr = pl.ds(hh * 8, 8)
                logits = [st[0, b] * SCALE for b in range(4)]
                for b in range(4):
                    a1 = st[1, b] * SCALE
                    prev = l1_s[b, hr, pl.ds(t0, 128)]
                    l1_s[b, hr, pl.ds(128 + t0, C)] = a1
                    xa = jnp.concatenate([prev, a1[:, :128]], axis=1)
                    logits.append(shr(xa, a1, 8))
                if c == 0:
                    pos = jax.lax.broadcasted_iota(jnp.int32, (8, C), 1)
                    logits = [jnp.where(pos >= 2 * w, l, -1e9) for w, l in enumerate(logits)]
                m = logits[0]
                for w in range(1, W):
                    m = jnp.maximum(m, logits[w])
                e = [jnp.exp(l - m) for l in logits]
                den = e[0]
                for w in range(1, W):
                    den = den + e[w]
                inv = 1.0 / den
                for w in range(W):
                    p_s[w, hr, pl.ds(t0, C)] = e[w] * inv
            return step

        out = []
        for hh in range(2):
            out += [qk(hh, d) for d in range(DH)] + [softmax(hh)]
        return out

    def pv_pieces(c):
        t0 = c * C
        st = {}

        def load_p(hh):
            def step(tk):
                hr = pl.ds(hh * 8, 8)
                P = [p_s[w, hr, pl.ds(t0, C)] for w in range(4)]
                for b in range(4):
                    px = p_s[4 + b, hr, pl.ds(t0, C + 128)]
                    P.append(shl(px[:, :C], px[:, 128:], 8))
                st["P"] = P
            return step

        def pv(hh, d):
            def step(tk):
                P = st["P"]
                r = pl.ds(d * H + hh * 8, 8)
                vx = _gate_mid(v_s[r, pl.ds(t0, C + 128)], tk)
                o0 = None
                o1 = None
                for b in range(4):
                    vb = shr(vx[:, :C], vx[:, 128:], 2 * b)
                    a = P[b] * vb
                    bb = P[4 + b] * vb
                    o0 = a if b == 0 else o0 + a
                    o1 = bb if b == 0 else o1 + bb
                prev = o1c_s[c, r, :]
                if c + 1 < NC:
                    o1c_s[c + 1, r, :] = o1[:, 128:]
                xa = jnp.concatenate([prev, o1[:, :128]], axis=1)
                o_s[r, pl.ds(t0, C)] = o0 + shr(xa, o1, 8)
            return step

        out = []
        for hh in range(2):
            out += [load_p(hh)] + [pv(hh, d) for d in range(DH)]
        return out

    def final(c, pieces):
        cols = pl.ds(c * C, C)
        parts = split(pieces, 5)
        acc = None
        for i, (k0, k1) in enumerate(((0, 512), (512, 1024), (1024, 1536), (1536, F))):
            r = jnp.dot(cat(g, range(k0 // 128, k1 // 128)), cat(w2, (2 * c, 2 * c + 1), k0, k1 - k0),
                        preferred_element_type=F32)
            release(r, parts[i])
            acc = r if acc is None else acc + r
        a = jnp.dot(cat(woT, range(4)), o_s[:, cols].astype(BF), preferred_element_type=F32)
        release(a, parts[4])
        xr = cat(xT, (2 * c, 2 * c + 1)).astype(F32)
        res = (acc + a) + b2row[:, c * C:(c + 1) * C] + xr
        resb = res.astype(BF)
        for i, (r0, nr) in enumerate(out_blocks(c)):
            outb[2 * c, pl.ds(r0, nr), :] = resb[r0:r0 + nr, :128]
            outb[2 * c + 1, pl.ds(r0, nr), :] = resb[r0:r0 + nr, 128:]
            for cp in out_copies(c, r0, nr):
                cp.start()

    start("wq"); start("x0"); start("x1")
    zero_pads()
    wait("wq")
    start("wk"); start("wv")
    release(None, prep_wqkv_pieces(0))
    wait("x0")
    release(None, ln_steps(0, 2))
    qkv_dot(0, 0, [], 0, D // 2)
    wait("x1")
    start("x2")
    l23 = ln_steps(2, 4)
    qkv_dot(0, 0, l23, D // 2, D // 2)
    wait("wk")
    qkv_dot(1, 0, prep_wqkv_pieces(1))
    qkv_dot(0, 1, [])
    wait("wv")
    start("w1a")
    l45 = ln_steps(4, 6)
    qkv_dot(1, 1, prep_wqkv_pieces(2))
    qkv_dot(0, 2, l45[:29])
    qkv_dot(1, 2, l45[29:])
    wait("x2")
    start("w1b"); start("w2")
    att = {(c, s): [] for c in range(NC) for s in range(3)}
    for c in range(2, NC - 1):
        a, b, d_ = split(ln_steps(2 * c + 2, 2 * c + 4), 3)
        att[c, 0] += a
        att[c, 1] += b
        att[c, 2] += d_
    a, b, d_ = split(qk_pieces(0), 3)
    att[7, 0] += a
    att[7, 1] += b
    att[7, 2] += d_
    for c in range(2, NC):
        for s in range(3):
            qkv_dot(c, s, att[c, s])
    wait("w1a"); wait("w1b")
    b1row = b1[...].astype(F32).reshape(1, F)
    wo_ = split(prep_wo_pieces(), 4)
    pv0 = split(pv_pieces(0), 3)
    u_group(0, qk_pieces(1) + wo_[0])
    u_group(1, qk_pieces(2) + wo_[1])
    u_group(2, qk_pieces(3) + wo_[2])
    u_group(3, qk_pieces(4) + wo_[3])
    u_group(4, qk_pieces(5) + pv0[0])
    u_group(5, qk_pieces(6) + pv0[1])
    u_group(6, qk_pieces(7) + pv0[2], mid=lambda: wait("w2"))
    b2row = b2[...].astype(F32).reshape(1, S)
    fin = {c: [] for c in range(NC)}
    for c in range(NC - 1):
        fin[c] += pv_pieces(c + 1)
    for c in range(NC):
        final(c, fin[c])
    for c in range(NC):
        for r0, nr in out_blocks(c):
            for cp in out_copies(c, r0, nr):
                cp.wait()


def _call(xT, wqkv, wo, w1, b1, w2, b2):
    any_spec = pl.BlockSpec(memory_space=pl.ANY)
    scratch = [
        pltpu.VMEM((S // 128, D, 128), BF), pltpu.VMEM((D, 3 * D), BF), pltpu.VMEM((D, D), BF),
        pltpu.VMEM((F // 128, S, 128), BF), pltpu.VMEM((F,), BF), pltpu.VMEM((S // 128, F, 128), BF), pltpu.VMEM((S,), BF),
        pltpu.VMEM((S // 128, D, 128), BF),
        pltpu.VMEM((S // 128, 512, 128), BF),
        pltpu.VMEM((4, D, 128), F32),
        pltpu.VMEM((4, 672, 128), U32),
        pltpu.VMEM((4, 3 * D, 128), BF),
        pltpu.VMEM((4, D, 128), BF),
        pltpu.VMEM((F // 128, D, 128), BF),
        pltpu.VMEM((D, S + 128), F32),
        pltpu.VMEM((D, S + 128), F32),
        pltpu.VMEM((D, S + 128), F32),
        pltpu.VMEM((4, H, S + 128), F32),
        pltpu.VMEM((W, H, S + 128), F32),
        pltpu.VMEM((NC, D, 128), F32),
        pltpu.VMEM((512, S), F32),
        pltpu.VMEM((S // 128, D, 128), BF),
        pltpu.SemaphoreType.DMA((9 + NC,)),
    ]
    return pl.pallas_call(
        kernel,
        out_shape=jax.ShapeDtypeStruct((D, S), BF),
        in_specs=[any_spec] * 7,
        out_specs=any_spec,
        scratch_shapes=scratch,
        compiler_params=pltpu.CompilerParams(vmem_limit_bytes=110 * 1024 * 1024),
    )(xT, wqkv, wo, w1, b1, w2, b2)


@jax.jit
def pallas_parallel_sum__sliding_local_dilated__mixer_token_mlp__prompt_kernel(A_x, A_wqkv, A_wo, B_x, B_w1, B_b1, B_w2, B_b2):
    outT = _call(A_x[0].T, A_wqkv, A_wo, B_w1, B_b1, B_w2, B_b2)
    return outT.T[None]
```

```python
import jax
import jax.numpy as jnp
import jax.experimental.pallas as pl
import jax.experimental.pallas.tpu as pltpu

S, D, H, DH, F = 2048, 448, 16, 28, 1792
W = 8
C = 256
NC = S // C
NG = 256
NJ = F // NG
EPS = 1e-5
SCALE = DH ** -0.5
BF, F32, U32 = jnp.bfloat16, jnp.float32, jnp.uint32
NTOK = 8
LN_RB = 32


def _gelu(x):
    c0 = 0.7978845608028654
    inner = c0 * (x + 0.044715 * (x * x * x))
    return 0.5 * x * (1.0 + jnp.tanh(inner))


def _rot256(y, shift):
    return jnp.concatenate(
        [pltpu.roll(y[:, :128], shift, axis=1), pltpu.roll(y[:, 128:], shift, axis=1)], axis=1)


def _tok(v):
    return (pltpu.bitcast(v[0:8, 0:128], U32) >> 31) >> 1


def _gate_f32(x, tk):
    if tk is None:
        return x
    t = jnp.tile(tk, (x.shape[0] // 8, x.shape[1] // 128))
    return jax.lax.bitcast_convert_type(pltpu.bitcast(x, U32) | t, F32)


def _gate(wd, tk):
    if tk is None:
        return wd
    return wd | jnp.tile(tk, (wd.shape[0] // 8, wd.shape[1] // 128))


def _gate_mid(x, tk):
    if tk is None:
        return x
    return jnp.concatenate([x[:, :128], _gate_f32(x[:, 128:256], tk), x[:, 256:]], axis=1)


def _gate_words(xb, tk):
    wd = pltpu.bitcast(xb, U32)
    if tk is None:
        return wd
    return wd | jnp.tile(tk, (wd.shape[0] // 8, wd.shape[1] // 128))


def kernel(xT_hbm, wqkv_hbm, wo_hbm, w1_hbm, b1_hbm, w2_hbm, b2_hbm, out_hbm,
           xT, wqkv, wo, w1, b1, w2, b2,
           hT, xnT, tmpT, tmpU, wqkvT, woT, g,
           q_s, k_s, v_s, l1_s, p_s, o1c_s, o_s, outb, sems):
    lane256 = jax.lax.broadcasted_iota(jnp.int32, (8, C), 1) % 128

    groups = {}

    def add(gname, src, dst):
        if gname not in groups:
            groups[gname] = (len(groups), [])
        idx, lst = groups[gname]
        lst.append(pltpu.make_async_copy(src, dst, sems.at[idx]))

    def add_x(gname, t0, t1):
        for a0 in range(t0, t1, 128):
            add(gname, xT_hbm.at[:, pl.ds(a0, 128)], xT.at[a0 // 128])

    def add_w1(gname, r0, r1, c0, c1, step):
        for j in range(c0 // 128, c1 // 128):
            for a0 in range(r0, r1, step):
                add(gname, w1_hbm.at[pl.ds(a0, step), pl.ds(j * 128, 128)], w1.at[j, pl.ds(a0, step), :])

    def add_rows(gname, src, dst, step):
        for a0 in range(0, src.shape[0], step):
            add(gname, src.at[pl.ds(a0, step), :], dst.at[pl.ds(a0, step), :])

    def start(gname):
        for cp in groups[gname][1]:
            cp.start()

    def wait(gname):
        for cp in groups[gname][1]:
            cp.wait()

    def add_cols(gname, src_, dst, c0, c1, rstep):
        for a0 in range(0, src_.shape[0], rstep):
            add(gname, src_.at[pl.ds(a0, rstep), pl.ds(c0, c1 - c0)], dst.at[pl.ds(a0, rstep), pl.ds(c0, c1 - c0)])

    add_cols("wq", wqkv_hbm, wqkv, 0, 512, 224)
    add_x("x0", 0, 256)
    add_x("x1", 256, 512)
    add_cols("wk", wqkv_hbm, wqkv, 512, 896, 224)
    add_cols("wv", wqkv_hbm, wqkv, 896, 3 * D, 224)
    add_x("wv", 512, 768)
    add_x("x2", 768, S)
    for j in range(0, 4):
        add_w1("w1a", 0, S, j * NG, (j + 1) * NG, 1024)
    add("w1a", b1_hbm, b1)
    for j in range(4, NJ):
        add_w1("w1b", 0, S, j * NG, (j + 1) * NG, 1024)
    add_rows("w1b", wo_hbm, wo, 224)
    add("w2", b2_hbm, b2)
    for j in range(S // 128):
        for a0 in range(0, F, 896):
            add("w2", w2_hbm.at[pl.ds(a0, 896), pl.ds(j * 128, 128)], w2.at[j, pl.ds(a0, 896), :])
    n_in = len(groups)

    def out_blocks(c):
        return [(0, D)] if c + 1 < NC else [(r0, 112) for r0 in range(0, D, 112)]

    def out_copies(c, r0, nr):
        return [pltpu.make_async_copy(outb.at[2 * c + i, pl.ds(r0, nr), :],
                                      out_hbm.at[pl.ds(r0, nr), pl.ds((2 * c + i) * 128, 128)], sems.at[n_in + c])
                for i in range(2)]

    def cat(ref, tiles, r0=0, nr=None):
        nr = ref.shape[1] - r0 if nr is None else nr
        words = ref.bitcast(U32)
        return jnp.concatenate([pltpu.bitcast(words[t, pl.ds(r0 // 2, nr // 2), :], BF) for t in tiles], axis=1)

    def release(r, pieces, ntok=NTOK):
        n = len(pieces)
        done = 0
        for q in range(ntok):
            upto = (n * (q + 1)) // ntok
            if done < upto:
                tk = _tok(r[q * (r.shape[0] // ntok):, :]) if r is not None else None
                while done < upto:
                    pieces[done](tk)
                    done += 1

    def split(lst, n):
        return [lst[(len(lst) * i) // n:(len(lst) * (i + 1)) // n] for i in range(n)]

    xw = xT.bitcast(U32)

    def ln_pieces(t):
        RB = LN_RB
        st = {}

        def p1(r0):
            def step(tk):
                wd = _gate(xw[t, pl.ds(r0 // 2, RB // 2), :], tk)
                lo = jax.lax.bitcast_convert_type(wd << 16, F32)
                hi = jax.lax.bitcast_convert_type(wd & U32(0xFFFF0000), F32)
                if r0 == 0:
                    st["c"] = jnp.broadcast_to(lo[0:1, :], (RB // 2, 128))
                a = lo - st["c"]
                b = hi - st["c"]
                p = a + b
                q = a * a + b * b
                st["s1"] = p if r0 == 0 else st["s1"] + p
                st["s2"] = q if r0 == 0 else st["s2"] + q
            return step

        def stats(tk):
            s1 = jnp.sum(st["s1"], axis=0, keepdims=True) * (1.0 / D)
            s2 = jnp.sum(st["s2"], axis=0, keepdims=True) * (1.0 / D)
            st["m"] = st["c"][0:1] + s1
            v = s2 - s1 * s1
            r = jax.lax.rsqrt(v + EPS)
            st["r"] = r
            st["rr"] = r * jax.lax.rsqrt(v * (r * r) + EPS)

        def p2(r0):
            def step(tk):
                wd = _gate(xw[t, pl.ds(r0 // 2, RB // 2), :], tk)
                xc = pltpu.bitcast(wd, BF).astype(F32) - st["m"]
                xnT[t, pl.ds(r0, RB), :] = (xc * st["r"]).astype(BF)
                hT[t, pl.ds(r0, RB), :] = (xc * st["rr"]).astype(BF)
            return step

        return [p1(r0) for r0 in range(0, D, RB)] + [stats] + [p2(r0) for r0 in range(0, D, RB)]

    def ln_steps(t0, t1):
        return [s for t in range(t0, t1) for s in ln_pieces(t)]

    def h_cols(t0, t1):
        return cat(hT, range(t0 // 128, t1 // 128))

    def u_group(j, pieces=(), mid=None):
        parts = split(list(pieces), 4)
        acc = None
        for i in range(4):
            if i == 2 and mid is not None:
                mid()
            r = jnp.dot(h_cols(i * 512, (i + 1) * 512), cat(w1, (2 * j, 2 * j + 1), i * 512, 512), preferred_element_type=F32)
            release(r, parts[i])
            acc = r if acc is None else acc + r
        act = _gelu(acc + b1row[:, j * NG:(j + 1) * NG]).astype(BF)
        g[2 * j] = act[:, :128]
        g[2 * j + 1] = act[:, 128:]

    def prep_wqkv_pieces(sec):
        def tr(kt, ct):
            rows = 128 if kt < 3 else 64
            cols = 128 if ct < 10 else 64

            def step(tk):
                blk = wqkv[pl.ds(kt * 128, rows), pl.ds(ct * 128, cols)]
                if tk is not None and cols == 128:
                    blk = pltpu.bitcast(_gate_words(blk, tk), BF)
                tmpU[kt, pl.ds(ct * 64, cols // 2), pl.ds(0, rows)] = pltpu.bitcast(blk.T, U32)
            return step

        def ga(kt, d0):
            def step(tk):
                for d in range(d0, d0 + 4, 2):
                    wd = tmpU[kt, pl.ds((sec * D + d) // 2, H, stride=DH // 2), :]
                    if tk is not None:
                        wd = wd | jnp.tile(tk, (2, 1))
                    lo = jax.lax.bitcast_convert_type(wd << 16, F32)
                    hi = jax.lax.bitcast_convert_type(wd & U32(0xFFFF0000), F32)
                    wqkvT[kt, pl.ds(sec * D + d * H, H), :] = lo.astype(BF)
                    wqkvT[kt, pl.ds(sec * D + (d + 1) * H, H), :] = hi.astype(BF)
            return step

        c_lo = (sec * D) // 128
        c_hi = (sec * D + D - 1) // 128
        if sec > 0:
            c_lo += 1 if sec * D % 128 else 0
        a = [tr(kt, ct) for ct in range(c_lo, c_hi + 1) for kt in range(4)]
        b = [ga(kt, d0) for kt in range(4) for d0 in range(0, DH, 4)]
        return a + b

    def prep_wo_pieces():
        def cp(et, r0):
            cols = 128 if et < 3 else 64

            def step(tk):
                blk = wo[pl.ds(r0, 112), pl.ds(et * 128, cols)]
                if tk is not None and cols == 128:
                    blk = pltpu.bitcast(_gate_words(blk, tk), BF)
                tmpT[et, pl.ds(r0, 112), pl.ds(0, cols)] = blk.astype(F32)
            return step

        def ga(et, ct):
            ecols = 128 if et < 3 else 64
            nd = 8 if ct < 3 else 4

            def step(tk):
                planes = [_gate_f32(tmpT[et, pl.ds(ct * 8 + dd, H, stride=DH), :], tk) for dd in range(nd)]
                if nd < 8:
                    planes.append(jnp.zeros(((8 - nd) * H, 128), F32))
                blk = jnp.concatenate(planes, axis=0)
                woT[ct, pl.ds(et * 128, ecols), :] = blk.T[:ecols, :].astype(BF)
            return step

        a = [cp(et, r0) for et in range(4) for r0 in range(0, D, 112)]
        b = [ga(et, ct) for et in range(4) for ct in range(4)]
        return a + b

    def zero_pads():
        xnT[:, pl.ds(D, 64), :] = jnp.zeros((S // 128, 64, 128), BF)
        o_s[pl.ds(D, 64), :] = jnp.zeros((64, S), F32)
        q_s[:, pl.ds(S, 128)] = jnp.zeros((D, 128), F32)
        k_s[:, pl.ds(0, 128)] = jnp.zeros((D, 128), F32)
        v_s[:, pl.ds(0, 128)] = jnp.zeros((D, 128), F32)
        for b in range(4):
            l1_s[b, :, pl.ds(0, 128)] = jnp.zeros((H, 128), F32)
            p_s[4 + b, :, pl.ds(S, 128)] = jnp.zeros((H, 128), F32)
        o1c_s[0] = jnp.zeros((D, 128), F32)
        tmpU[3] = jnp.zeros((672, 128), U32)
        tmpT[3] = jnp.zeros((D, 128), F32)

    def qkv_dot(c, sec, pieces, r0=0, nr=D):
        rhs = cat(xnT, (2 * c, 2 * c + 1))
        r = jnp.dot(cat(wqkvT, range(4), sec * D + r0, nr), rhs, preferred_element_type=F32)
        dst, off = ((q_s, 0), (k_s, 128), (v_s, 128))[sec]
        dst[pl.ds(r0, nr), pl.ds(off + c * C, C)] = r
        release(r, pieces)

    def shr(xa, xb, n):
        if n == 0:
            return xb
        return _rot256(jnp.where(lane256 >= 128 - n, xa, xb), n)

    def shl(xa, xb, n):
        return _rot256(jnp.where(lane256 < n, xb, xa), 128 - n)

    def qk_pieces(c):
        t0 = c * C
        st = {}

        def qk(hh, d):
            def step(tk):
                r = pl.ds(d * H + hh * 8, 8)
                qx = _gate_mid(q_s[r, pl.ds(t0, C + 128)], tk)
                kx = _gate_mid(k_s[r, pl.ds(t0, C + 128)], tk)
                q0 = qx[:, :C]
                q1 = shl(qx[:, :C], qx[:, 128:], 8)
                for b in range(4):
                    kb = shr(kx[:, :C], kx[:, 128:], 2 * b)
                    p0 = q0 * kb
                    p1 = q1 * kb
                    st[0, b] = p0 if d == 0 else st[0, b] + p0
                    st[1, b] = p1 if d == 0 else st[1, b] + p1
            return step

        def softmax(hh):
            def step(tk):
                hr = pl.ds(hh * 8, 8)
                logits = [st[0, b] * SCALE for b in range(4)]
                for b in range(4):
                    a1 = st[1, b] * SCALE
                    prev = l1_s[b, hr, pl.ds(t0, 128)]
                    l1_s[b, hr, pl.ds(128 + t0, C)] = a1
                    xa = jnp.concatenate([prev, a1[:, :128]], axis=1)
                    logits.append(shr(xa, a1, 8))
                if c == 0:
                    pos = jax.lax.broadcasted_iota(jnp.int32, (8, C), 1)
                    logits = [jnp.where(pos >= 2 * w, l, -1e9) for w, l in enumerate(logits)]
                m = logits[0]
                for w in range(1, W):
                    m = jnp.maximum(m, logits[w])
                e = [jnp.exp(l - m) for l in logits]
                den = e[0]
                for w in range(1, W):
                    den = den + e[w]
                inv = 1.0 / den
                for w in range(W):
                    p_s[w, hr, pl.ds(t0, C)] = e[w] * inv
            return step

        out = []
        for hh in range(2):
            out += [qk(hh, d) for d in range(DH)] + [softmax(hh)]
        return out

    def pv_pieces(c):
        t0 = c * C
        st = {}

        def load_p(hh):
            def step(tk):
                hr = pl.ds(hh * 8, 8)
                P = [p_s[w, hr, pl.ds(t0, C)] for w in range(4)]
                for b in range(4):
                    px = p_s[4 + b, hr, pl.ds(t0, C + 128)]
                    P.append(shl(px[:, :C], px[:, 128:], 8))
                st["P"] = P
            return step

        def pv(hh, d):
            def step(tk):
                P = st["P"]
                r = pl.ds(d * H + hh * 8, 8)
                vx = _gate_mid(v_s[r, pl.ds(t0, C + 128)], tk)
                o0 = None
                o1 = None
                for b in range(4):
                    vb = shr(vx[:, :C], vx[:, 128:], 2 * b)
                    a = P[b] * vb
                    bb = P[4 + b] * vb
                    o0 = a if b == 0 else o0 + a
                    o1 = bb if b == 0 else o1 + bb
                prev = o1c_s[c, r, :]
                if c + 1 < NC:
                    o1c_s[c + 1, r, :] = o1[:, 128:]
                xa = jnp.concatenate([prev, o1[:, :128]], axis=1)
                o_s[r, pl.ds(t0, C)] = o0 + shr(xa, o1, 8)
            return step

        out = []
        for hh in range(2):
            out += [load_p(hh)] + [pv(hh, d) for d in range(DH)]
        return out

    def final(c, pieces):
        cols = pl.ds(c * C, C)
        parts = split(pieces, 5)
        acc = None
        for i, (k0, k1) in enumerate(((0, 512), (512, 1024), (1024, 1536), (1536, F))):
            r = jnp.dot(cat(g, range(k0 // 128, k1 // 128)), cat(w2, (2 * c, 2 * c + 1), k0, k1 - k0),
                        preferred_element_type=F32)
            release(r, parts[i])
            acc = r if acc is None else acc + r
        a = jnp.dot(cat(woT, range(4)), o_s[:, cols].astype(BF), preferred_element_type=F32)
        release(a, parts[4])
        xr = cat(xT, (2 * c, 2 * c + 1)).astype(F32)
        res = (acc + a) + b2row[:, c * C:(c + 1) * C] + xr
        resb = res.astype(BF)
        for i, (r0, nr) in enumerate(out_blocks(c)):
            outb[2 * c, pl.ds(r0, nr), :] = resb[r0:r0 + nr, :128]
            outb[2 * c + 1, pl.ds(r0, nr), :] = resb[r0:r0 + nr, 128:]
            for cp in out_copies(c, r0, nr):
                cp.start()

    start("wq"); start("x0"); start("x1")
    zero_pads()
    wait("wq")
    start("wk"); start("wv")
    release(None, prep_wqkv_pieces(0))
    wait("x0")
    release(None, ln_steps(0, 2))
    qkv_dot(0, 0, [], 0, D // 2)
    wait("x1")
    start("x2")
    l23 = ln_steps(2, 4)
    qkv_dot(0, 0, l23, D // 2, D // 2)
    wait("wk")
    qkv_dot(1, 0, prep_wqkv_pieces(1))
    qkv_dot(0, 1, [])
    wait("wv")
    start("w1a")
    l45 = ln_steps(4, 6)
    qkv_dot(1, 1, prep_wqkv_pieces(2))
    qkv_dot(0, 2, l45[:29])
    qkv_dot(1, 2, l45[29:])
    wait("x2")
    start("w1b"); start("w2")
    att = {(c, s): [] for c in range(NC) for s in range(3)}
    for c in range(2, NC - 1):
        a, b, d_ = split(ln_steps(2 * c + 2, 2 * c + 4), 3)
        att[c, 0] += a
        att[c, 1] += b
        att[c, 2] += d_
    a, b, d_ = split(qk_pieces(0), 3)
    att[7, 0] += a
    att[7, 1] += b
    att[7, 2] += d_
    for c in range(2, NC):
        for s in range(3):
            qkv_dot(c, s, att[c, s])
    wait("w1a"); wait("w1b")
    b1row = b1[...].astype(F32).reshape(1, F)
    wo_ = split(prep_wo_pieces(), 4)
    pv0 = split(pv_pieces(0), 3)
    u_group(0, qk_pieces(1) + wo_[0])
    u_group(1, qk_pieces(2) + wo_[1])
    u_group(2, qk_pieces(3) + wo_[2])
    u_group(3, qk_pieces(4) + wo_[3])
    u_group(4, qk_pieces(5) + pv0[0])
    u_group(5, qk_pieces(6) + pv0[1])
    u_group(6, qk_pieces(7) + pv0[2], mid=lambda: wait("w2"))
    b2row = b2[...].astype(F32).reshape(1, S)
    for c in range(NC):
        final(c, pv_pieces(c + 1) if c + 1 < NC else [])
    for c in range(NC):
        for r0, nr in out_blocks(c):
            for cp in out_copies(c, r0, nr):
                cp.wait()


def _call(xT, wqkv, wo, w1, b1, w2, b2):
    any_spec = pl.BlockSpec(memory_space=pl.ANY)
    scratch = [
        pltpu.VMEM((S // 128, D, 128), BF), pltpu.VMEM((D, 3 * D), BF), pltpu.VMEM((D, D), BF),
        pltpu.VMEM((F // 128, S, 128), BF), pltpu.VMEM((F,), BF), pltpu.VMEM((S // 128, F, 128), BF), pltpu.VMEM((S,), BF),
        pltpu.VMEM((S // 128, D, 128), BF),
        pltpu.VMEM((S // 128, 512, 128), BF),
        pltpu.VMEM((4, D, 128), F32),
        pltpu.VMEM((4, 672, 128), U32),
        pltpu.VMEM((4, 3 * D, 128), BF),
        pltpu.VMEM((4, D, 128), BF),
        pltpu.VMEM((F // 128, D, 128), BF),
        pltpu.VMEM((D, S + 128), F32),
        pltpu.VMEM((D, S + 128), F32),
        pltpu.VMEM((D, S + 128), F32),
        pltpu.VMEM((4, H, S + 128), F32),
        pltpu.VMEM((W, H, S + 128), F32),
        pltpu.VMEM((NC, D, 128), F32),
        pltpu.VMEM((512, S), F32),
        pltpu.VMEM((S // 128, D, 128), BF),
        pltpu.SemaphoreType.DMA((9 + NC,)),
    ]
    return pl.pallas_call(
        kernel,
        out_shape=jax.ShapeDtypeStruct((D, S), BF),
        in_specs=[any_spec] * 7,
        out_specs=any_spec,
        scratch_shapes=scratch,
        compiler_params=pltpu.CompilerParams(vmem_limit_bytes=110 * 1024 * 1024),
    )(xT, wqkv, wo, w1, b1, w2, b2)


@jax.jit
def pallas_parallel_sum__sliding_local_dilated__mixer_token_mlp__prompt_kernel(A_x, A_wqkv, A_wo, B_x, B_w1, B_b1, B_w2, B_b2):
    outT = _call(A_x[0].T, A_wqkv, A_wo, B_w1, B_b1, B_w2, B_b2)
    return outT.T[None]
```

```python
import jax
import jax.numpy as jnp
import jax.experimental.pallas as pl
import jax.experimental.pallas.tpu as pltpu

S, D, H, DH, F = 2048, 448, 16, 28, 1792
W = 8
C = 256
NC = S // C
NG = 256
NJ = F // NG
EPS = 1e-5
SCALE = DH ** -0.5
BF, F32, U32 = jnp.bfloat16, jnp.float32, jnp.uint32
NTOK = 8
LN_RB = 32


def _gelu(x):
    c0 = 0.7978845608028654
    inner = c0 * (x + 0.044715 * (x * x * x))
    return 0.5 * x * (1.0 + jnp.tanh(inner))


def _rot256(y, shift):
    return jnp.concatenate(
        [pltpu.roll(y[:, :128], shift, axis=1), pltpu.roll(y[:, 128:], shift, axis=1)], axis=1)


def _tok(v):
    return (pltpu.bitcast(v[0:8, 0:128], U32) >> 31) >> 1


def _gate_f32(x, tk):
    if tk is None:
        return x
    t = jnp.tile(tk, (x.shape[0] // 8, x.shape[1] // 128))
    return jax.lax.bitcast_convert_type(pltpu.bitcast(x, U32) | t, F32)


def _gate(wd, tk):
    if tk is None:
        return wd
    return wd | jnp.tile(tk, (wd.shape[0] // 8, wd.shape[1] // 128))


def _gate_mid(x, tk):
    if tk is None:
        return x
    return jnp.concatenate([x[:, :128], _gate_f32(x[:, 128:256], tk), x[:, 256:]], axis=1)


def _gate_words(xb, tk):
    wd = pltpu.bitcast(xb, U32)
    if tk is None:
        return wd
    return wd | jnp.tile(tk, (wd.shape[0] // 8, wd.shape[1] // 128))


def kernel(xT_hbm, wqkv_hbm, wo_hbm, w1_hbm, b1_hbm, w2_hbm, b2_hbm, out_hbm,
           xT, wqkv, wo, w1, b1, w2, b2,
           hT, xnT, tmpT, tmpU, wqkvT, woT, g,
           q_s, k_s, v_s, l1_s, p_s, o1c_s, o_s, outb, sems):
    lane256 = jax.lax.broadcasted_iota(jnp.int32, (8, C), 1) % 128

    groups = {}

    def add(gname, src, dst):
        if gname not in groups:
            groups[gname] = (len(groups), [])
        idx, lst = groups[gname]
        lst.append(pltpu.make_async_copy(src, dst, sems.at[idx]))

    def add_x(gname, t0, t1):
        for a0 in range(t0, t1, 128):
            add(gname, xT_hbm.at[:, pl.ds(a0, 128)], xT.at[a0 // 128])

    def add_w1(gname, r0, r1, c0, c1, step):
        for j in range(c0 // 128, c1 // 128):
            for a0 in range(r0, r1, step):
                add(gname, w1_hbm.at[pl.ds(a0, step), pl.ds(j * 128, 128)], w1.at[j, pl.ds(a0, step), :])

    def add_rows(gname, src, dst, step):
        for a0 in range(0, src.shape[0], step):
            add(gname, src.at[pl.ds(a0, step), :], dst.at[pl.ds(a0, step), :])

    def start(gname):
        for cp in groups[gname][1]:
            cp.start()

    def wait(gname):
        for cp in groups[gname][1]:
            cp.wait()

    def add_cols(gname, src_, dst, c0, c1, rstep):
        for a0 in range(0, src_.shape[0], rstep):
            add(gname, src_.at[pl.ds(a0, rstep), pl.ds(c0, c1 - c0)], dst.at[pl.ds(a0, rstep), pl.ds(c0, c1 - c0)])

    add_cols("wq", wqkv_hbm, wqkv, 0, 512, 224)
    add_x("x0", 0, 256)
    add_x("x1", 256, 512)
    add_cols("wk", wqkv_hbm, wqkv, 512, 896, 224)
    add_cols("wv", wqkv_hbm, wqkv, 896, 3 * D, 224)
    add_x("wv", 512, 768)
    add_x("x2", 768, S)
    for j in range(0, 4):
        add_w1("w1a", 0, S, j * NG, (j + 1) * NG, 1024)
    add("w1a", b1_hbm, b1)
    for j in range(4, NJ):
        add_w1("w1b", 0, S, j * NG, (j + 1) * NG, 1024)
    add_rows("w1b", wo_hbm, wo, 224)
    add("w2", b2_hbm, b2)
    for j in range(S // 128):
        for a0 in range(0, F, 896):
            add("w2", w2_hbm.at[pl.ds(a0, 896), pl.ds(j * 128, 128)], w2.at[j, pl.ds(a0, 896), :])
    n_in = len(groups)

    def out_blocks(c):
        return [(0, D)] if c + 1 < NC else [(r0, 112) for r0 in range(0, D, 112)]

    def out_copies(c, r0, nr):
        return [pltpu.make_async_copy(outb.at[2 * c + i, pl.ds(r0, nr), :],
                                      out_hbm.at[pl.ds(r0, nr), pl.ds((2 * c + i) * 128, 128)], sems.at[n_in + c])
                for i in range(2)]

    def cat(ref, tiles, r0=0, nr=None):
        nr = ref.shape[1] - r0 if nr is None else nr
        words = ref.bitcast(U32)
        return jnp.concatenate([pltpu.bitcast(words[t, pl.ds(r0 // 2, nr // 2), :], BF) for t in tiles], axis=1)

    def release(r, pieces, ntok=NTOK):
        n = len(pieces)
        done = 0
        for q in range(ntok):
            upto = (n * (q + 1)) // ntok
            if done < upto:
                tk = _tok(r[q * (r.shape[0] // ntok):, :]) if r is not None else None
                while done < upto:
                    pieces[done](tk)
                    done += 1

    def split(lst, n):
        return [lst[(len(lst) * i) // n:(len(lst) * (i + 1)) // n] for i in range(n)]

    xw = xT.bitcast(U32)

    def ln_pieces(t):
        RB = LN_RB
        st = {}

        def p1(r0):
            def step(tk):
                wd = _gate(xw[t, pl.ds(r0 // 2, RB // 2), :], tk)
                lo = jax.lax.bitcast_convert_type(wd << 16, F32)
                hi = jax.lax.bitcast_convert_type(wd & U32(0xFFFF0000), F32)
                if r0 == 0:
                    st["c"] = jnp.broadcast_to(lo[0:1, :], (RB // 2, 128))
                a = lo - st["c"]
                b = hi - st["c"]
                p = a + b
                q = a * a + b * b
                st["s1"] = p if r0 == 0 else st["s1"] + p
                st["s2"] = q if r0 == 0 else st["s2"] + q
            return step

        def stats(tk):
            s1 = jnp.sum(st["s1"], axis=0, keepdims=True) * (1.0 / D)
            s2 = jnp.sum(st["s2"], axis=0, keepdims=True) * (1.0 / D)
            st["m"] = st["c"][0:1] + s1
            v = s2 - s1 * s1
            r = jax.lax.rsqrt(v + EPS)
            mu = s1 - (st["m"] - st["c"][0:1])
            st["r"] = r
            st["rr"] = r * jax.lax.rsqrt((v - mu * mu) * (r * r) + EPS)
            st["beta"] = mu * st["rr"]

        def p2(r0):
            def step(tk):
                wd = _gate(xw[t, pl.ds(r0 // 2, RB // 2), :], tk)
                xc = pltpu.bitcast(wd, BF).astype(F32) - st["m"]
                xnT[t, pl.ds(r0, RB), :] = (xc * st["r"]).astype(BF)
                hT[t, pl.ds(r0, RB), :] = (xc * st["rr"] - st["beta"]).astype(BF)
            return step

        return [p1(r0) for r0 in range(0, D, RB)] + [stats] + [p2(r0) for r0 in range(0, D, RB)]

    def ln_steps(t0, t1):
        return [s for t in range(t0, t1) for s in ln_pieces(t)]

    def h_cols(t0, t1):
        return cat(hT, range(t0 // 128, t1 // 128))

    def u_group(j, pieces=(), mid=None):
        parts = split(list(pieces), 4)
        acc = None
        for i in range(4):
            if i == 2 and mid is not None:
                mid()
            r = jnp.dot(h_cols(i * 512, (i + 1) * 512), cat(w1, (2 * j, 2 * j + 1), i * 512, 512), preferred_element_type=F32)
            release(r, parts[i])
            acc = r if acc is None else acc + r
        act = _gelu(acc + b1row[:, j * NG:(j + 1) * NG]).astype(BF)
        g[2 * j] = act[:, :128]
        g[2 * j + 1] = act[:, 128:]

    def prep_wqkv_pieces(sec):
        def tr(kt, ct):
            rows = 128 if kt < 3 else 64
            cols = 128 if ct < 10 else 64

            def step(tk):
                blk = wqkv[pl.ds(kt * 128, rows), pl.ds(ct * 128, cols)]
                if tk is not None and cols == 128:
                    blk = pltpu.bitcast(_gate_words(blk, tk), BF)
                tmpU[kt, pl.ds(ct * 64, cols // 2), pl.ds(0, rows)] = pltpu.bitcast(blk.T, U32)
            return step

        def ga(kt, d0):
            def step(tk):
                for d in range(d0, d0 + 4, 2):
                    wd = tmpU[kt, pl.ds((sec * D + d) // 2, H, stride=DH // 2), :]
                    if tk is not None:
                        wd = wd | jnp.tile(tk, (2, 1))
                    lo = jax.lax.bitcast_convert_type(wd << 16, F32)
                    hi = jax.lax.bitcast_convert_type(wd & U32(0xFFFF0000), F32)
                    wqkvT[kt, pl.ds(sec * D + d * H, H), :] = lo.astype(BF)
                    wqkvT[kt, pl.ds(sec * D + (d + 1) * H, H), :] = hi.astype(BF)
            return step

        c_lo = (sec * D) // 128
        c_hi = (sec * D + D - 1) // 128
        if sec > 0:
            c_lo += 1 if sec * D % 128 else 0
        a = [tr(kt, ct) for ct in range(c_lo, c_hi + 1) for kt in range(4)]
        b = [ga(kt, d0) for kt in range(4) for d0 in range(0, DH, 4)]
        return a + b

    def prep_wo_pieces():
        def cp(et, r0):
            cols = 128 if et < 3 else 64

            def step(tk):
                blk = wo[pl.ds(r0, 112), pl.ds(et * 128, cols)]
                if tk is not None and cols == 128:
                    blk = pltpu.bitcast(_gate_words(blk, tk), BF)
                tmpT[et, pl.ds(r0, 112), pl.ds(0, cols)] = blk.astype(F32)
            return step

        def ga(et, ct):
            ecols = 128 if et < 3 else 64
            nd = 8 if ct < 3 else 4

            def step(tk):
                planes = [_gate_f32(tmpT[et, pl.ds(ct * 8 + dd, H, stride=DH), :], tk) for dd in range(nd)]
                if nd < 8:
                    planes.append(jnp.zeros(((8 - nd) * H, 128), F32))
                blk = jnp.concatenate(planes, axis=0)
                woT[ct, pl.ds(et * 128, ecols), :] = blk.T[:ecols, :].astype(BF)
            return step

        a = [cp(et, r0) for et in range(4) for r0 in range(0, D, 112)]
        b = [ga(et, ct) for et in range(4) for ct in range(4)]
        return a + b

    def zero_pads():
        xnT[:, pl.ds(D, 64), :] = jnp.zeros((S // 128, 64, 128), BF)
        o_s[pl.ds(D, 64), :] = jnp.zeros((64, S), F32)
        q_s[:, pl.ds(S, 128)] = jnp.zeros((D, 128), F32)
        k_s[:, pl.ds(0, 128)] = jnp.zeros((D, 128), F32)
        v_s[:, pl.ds(0, 128)] = jnp.zeros((D, 128), F32)
        for b in range(4):
            l1_s[b, :, pl.ds(0, 128)] = jnp.zeros((H, 128), F32)
            p_s[4 + b, :, pl.ds(S, 128)] = jnp.zeros((H, 128), F32)
        o1c_s[0] = jnp.zeros((D, 128), F32)
        tmpU[3] = jnp.zeros((672, 128), U32)
        tmpT[3] = jnp.zeros((D, 128), F32)

    def qkv_dot(c, sec, pieces, r0=0, nr=D):
        rhs = cat(xnT, (2 * c, 2 * c + 1))
        r = jnp.dot(cat(wqkvT, range(4), sec * D + r0, nr), rhs, preferred_element_type=F32)
        dst, off = ((q_s, 0), (k_s, 128), (v_s, 128))[sec]
        dst[pl.ds(r0, nr), pl.ds(off + c * C, C)] = r
        release(r, pieces)

    def shr(xa, xb, n):
        if n == 0:
            return xb
        return _rot256(jnp.where(lane256 >= 128 - n, xa, xb), n)

    def shl(xa, xb, n):
        return _rot256(jnp.where(lane256 < n, xb, xa), 128 - n)

    def qk_pieces(c):
        t0 = c * C
        st = {}

        def qk(hh, d):
            def step(tk):
                r = pl.ds(d * H + hh * 8, 8)
                qx = _gate_mid(q_s[r, pl.ds(t0, C + 128)], tk)
                kx = _gate_mid(k_s[r, pl.ds(t0, C + 128)], tk)
                q0 = qx[:, :C]
                q1 = shl(qx[:, :C], qx[:, 128:], 8)
                for b in range(4):
                    kb = shr(kx[:, :C], kx[:, 128:], 2 * b)
                    p0 = q0 * kb
                    p1 = q1 * kb
                    st[0, b] = p0 if d == 0 else st[0, b] + p0
                    st[1, b] = p1 if d == 0 else st[1, b] + p1
            return step

        def softmax(hh):
            def step(tk):
                hr = pl.ds(hh * 8, 8)
                logits = [st[0, b] * SCALE for b in range(4)]
                for b in range(4):
                    a1 = st[1, b] * SCALE
                    prev = l1_s[b, hr, pl.ds(t0, 128)]
                    l1_s[b, hr, pl.ds(128 + t0, C)] = a1
                    xa = jnp.concatenate([prev, a1[:, :128]], axis=1)
                    logits.append(shr(xa, a1, 8))
                if c == 0:
                    pos = jax.lax.broadcasted_iota(jnp.int32, (8, C), 1)
                    logits = [jnp.where(pos >= 2 * w, l, -1e9) for w, l in enumerate(logits)]
                m = logits[0]
                for w in range(1, W):
                    m = jnp.maximum(m, logits[w])
                e = [jnp.exp(l - m) for l in logits]
                den = e[0]
                for w in range(1, W):
                    den = den + e[w]
                inv = 1.0 / den
                for w in range(W):
                    p_s[w, hr, pl.ds(t0, C)] = e[w] * inv
            return step

        out = []
        for hh in range(2):
            out += [qk(hh, d) for d in range(DH)] + [softmax(hh)]
        return out

    def pv_pieces(c):
        t0 = c * C
        st = {}

        def load_p(hh):
            def step(tk):
                hr = pl.ds(hh * 8, 8)
                P = [p_s[w, hr, pl.ds(t0, C)] for w in range(4)]
                for b in range(4):
                    px = p_s[4 + b, hr, pl.ds(t0, C + 128)]
                    P.append(shl(px[:, :C], px[:, 128:], 8))
                st["P"] = P
            return step

        def pv(hh, d):
            def step(tk):
                P = st["P"]
                r = pl.ds(d * H + hh * 8, 8)
                vx = _gate_mid(v_s[r, pl.ds(t0, C + 128)], tk)
                o0 = None
                o1 = None
                for b in range(4):
                    vb = shr(vx[:, :C], vx[:, 128:], 2 * b)
                    a = P[b] * vb
                    bb = P[4 + b] * vb
                    o0 = a if b == 0 else o0 + a
                    o1 = bb if b == 0 else o1 + bb
                prev = o1c_s[c, r, :]
                if c + 1 < NC:
                    o1c_s[c + 1, r, :] = o1[:, 128:]
                xa = jnp.concatenate([prev, o1[:, :128]], axis=1)
                o_s[r, pl.ds(t0, C)] = o0 + shr(xa, o1, 8)
            return step

        out = []
        for hh in range(2):
            out += [load_p(hh)] + [pv(hh, d) for d in range(DH)]
        return out

    def final(c, pieces):
        cols = pl.ds(c * C, C)
        parts = split(pieces, 5)
        acc = None
        for i, (k0, k1) in enumerate(((0, 512), (512, 1024), (1024, 1536), (1536, F))):
            r = jnp.dot(cat(g, range(k0 // 128, k1 // 128)), cat(w2, (2 * c, 2 * c + 1), k0, k1 - k0),
                        preferred_element_type=F32)
            release(r, parts[i])
            acc = r if acc is None else acc + r
        a = jnp.dot(cat(woT, range(4)), o_s[:, cols].astype(BF), preferred_element_type=F32)
        release(a, parts[4])
        xr = cat(xT, (2 * c, 2 * c + 1)).astype(F32)
        res = (acc + a) + b2row[:, c * C:(c + 1) * C] + xr
        resb = res.astype(BF)
        for i, (r0, nr) in enumerate(out_blocks(c)):
            outb[2 * c, pl.ds(r0, nr), :] = resb[r0:r0 + nr, :128]
            outb[2 * c + 1, pl.ds(r0, nr), :] = resb[r0:r0 + nr, 128:]
            for cp in out_copies(c, r0, nr):
                cp.start()

    start("wq"); start("x0"); start("x1")
    zero_pads()
    wait("wq")
    start("wk"); start("wv")
    release(None, prep_wqkv_pieces(0))
    wait("x0")
    release(None, ln_steps(0, 2))
    qkv_dot(0, 0, [], 0, D // 2)
    wait("x1")
    start("x2")
    l23 = ln_steps(2, 4)
    qkv_dot(0, 0, l23, D // 2, D // 2)
    wait("wk")
    qkv_dot(1, 0, prep_wqkv_pieces(1))
    qkv_dot(0, 1, [])
    wait("wv")
    start("w1a")
    l45 = ln_steps(4, 6)
    qkv_dot(1, 1, prep_wqkv_pieces(2))
    qkv_dot(0, 2, l45[:29])
    qkv_dot(1, 2, l45[29:])
    wait("x2")
    start("w1b"); start("w2")
    att = {(c, s): [] for c in range(NC) for s in range(3)}
    for c in range(2, NC - 1):
        a, b, d_ = split(ln_steps(2 * c + 2, 2 * c + 4), 3)
        att[c, 0] += a
        att[c, 1] += b
        att[c, 2] += d_
    a, b, d_ = split(qk_pieces(0), 3)
    att[7, 0] += a
    att[7, 1] += b
    att[7, 2] += d_
    for c in range(2, NC):
        for s in range(3):
            qkv_dot(c, s, att[c, s])
    wait("w1a"); wait("w1b")
    b1row = b1[...].astype(F32).reshape(1, F)
    wo_ = split(prep_wo_pieces(), 4)
    pv0 = split(pv_pieces(0), 3)
    u_group(0, qk_pieces(1) + wo_[0])
    u_group(1, qk_pieces(2) + wo_[1])
    u_group(2, qk_pieces(3) + wo_[2])
    u_group(3, qk_pieces(4) + wo_[3])
    u_group(4, qk_pieces(5) + pv0[0])
    u_group(5, qk_pieces(6) + pv0[1])
    u_group(6, qk_pieces(7) + pv0[2], mid=lambda: wait("w2"))
    b2row = b2[...].astype(F32).reshape(1, S)
    for c in range(NC):
        final(c, pv_pieces(c + 1) if c + 1 < NC else [])
    for c in range(NC):
        for r0, nr in out_blocks(c):
            for cp in out_copies(c, r0, nr):
                cp.wait()


def _call(xT, wqkv, wo, w1, b1, w2, b2):
    any_spec = pl.BlockSpec(memory_space=pl.ANY)
    scratch = [
        pltpu.VMEM((S // 128, D, 128), BF), pltpu.VMEM((D, 3 * D), BF), pltpu.VMEM((D, D), BF),
        pltpu.VMEM((F // 128, S, 128), BF), pltpu.VMEM((F,), BF), pltpu.VMEM((S // 128, F, 128), BF), pltpu.VMEM((S,), BF),
        pltpu.VMEM((S // 128, D, 128), BF),
        pltpu.VMEM((S // 128, 512, 128), BF),
        pltpu.VMEM((4, D, 128), F32),
        pltpu.VMEM((4, 672, 128), U32),
        pltpu.VMEM((4, 3 * D, 128), BF),
        pltpu.VMEM((4, D, 128), BF),
        pltpu.VMEM((F // 128, D, 128), BF),
        pltpu.VMEM((D, S + 128), F32),
        pltpu.VMEM((D, S + 128), F32),
        pltpu.VMEM((D, S + 128), F32),
        pltpu.VMEM((4, H, S + 128), F32),
        pltpu.VMEM((W, H, S + 128), F32),
        pltpu.VMEM((NC, D, 128), F32),
        pltpu.VMEM((512, S), F32),
        pltpu.VMEM((S // 128, D, 128), BF),
        pltpu.SemaphoreType.DMA((9 + NC,)),
    ]
    return pl.pallas_call(
        kernel,
        out_shape=jax.ShapeDtypeStruct((D, S), BF),
        in_specs=[any_spec] * 7,
        out_specs=any_spec,
        scratch_shapes=scratch,
        compiler_params=pltpu.CompilerParams(vmem_limit_bytes=110 * 1024 * 1024),
    )(xT, wqkv, wo, w1, b1, w2, b2)


@jax.jit
def pallas_parallel_sum__sliding_local_dilated__mixer_token_mlp__prompt_kernel(A_x, A_wqkv, A_wo, B_x, B_w1, B_b1, B_w2, B_b2):
    outT = _call(A_x[0].T, A_wqkv, A_wo, B_w1, B_b1, B_w2, B_b2)
    return outT.T[None]
```
